```python
import os as _os
_os.environ.setdefault("JAX_PLATFORMS", "cpu")
import jax
import jax.numpy as jnp

def _softmax(x, axis=-1):
    return jax.nn.softmax(x, axis=axis)
def _gelu(x):
    return jax.nn.gelu(x, approximate=True)
def _silu(x):
    return jax.nn.silu(x)
def _sigmoid(x):
    return jax.nn.sigmoid(x)
def _layernorm(x, axis=-1, eps=1e-5):
    m = jnp.mean(x, axis=axis, keepdims=True)
    v = jnp.var(x, axis=axis, keepdims=True)
    return (x - m) / jnp.sqrt(v + eps)
def _scatter_add(tgt, idx, src, axis=0):
    return tgt.at[idx].add(src)
def _segment_sum(src, seg, n):
    return jax.ops.segment_sum(src, seg, n)
class _Rng:
    def __init__(self, key):
        self._k = key
    def _next(self):
        self._k, sub = jax.random.split(self._k)
        return sub
    def normal(self, shape):
        return jax.random.normal(self._next(), shape, dtype=jnp.bfloat16)
    def randint(self, lo, hi, shape):
        return jax.random.randint(self._next(), shape, lo, hi, dtype=jnp.int32)
    def uniform(self, shape, lo=0.0, hi=1.0):
        return jax.random.uniform(self._next(), shape, jnp.bfloat16, lo, hi)
    def permutation(self, n):
        return jax.random.permutation(self._next(), n)


kernel_name = 'sequential_preLN__softmax_full_mha__geglu_ffn__prompt'

def setup_inputs():
    _rng = _Rng(jax.random.key(int.from_bytes(__import__("os").urandom(4), "little")))
    _w = (lambda a: (lambda t: t.astype(jnp.bfloat16) if jnp.issubdtype(t.dtype, jnp.floating) else t)(jnp.asarray(a)))
    def _A_setup():
        B, S, D = 1, 2048, 512
        return {
            "x": _w((lambda *s: _rng.normal(s) * 0.05)(B, S, D)),
            "wqkv": _w((lambda *s: _rng.normal(s) * 0.05)(D, 3 * D)),
            "wo": _w((lambda *s: _rng.normal(s) * 0.05)(D, D)),
        }
    _A_in = _A_setup()

    def _B_setup():
        B, S, D, F = 1, 2048, 512, 1376
        return {
            "x": _w((lambda *s: _rng.normal(s) * 0.05)(B, S, D)),
            "w_gate": _w((lambda *s: _rng.normal(s) * 0.05)(D, F)),
            "w_up": _w((lambda *s: _rng.normal(s) * 0.05)(D, F)),
            "w_down": _w((lambda *s: _rng.normal(s) * 0.05)(F, D)),
        }
    _B_in = _B_setup()

    return {
        "A_x": _A_in["x"],
        "A_wqkv": _A_in["wqkv"],
        "A_wo": _A_in["wo"],
        "B_x": _B_in["x"],
        "B_w_gate": _B_in["w_gate"],
        "B_w_up": _B_in["w_up"],
        "B_w_down": _B_in["w_down"],
    }

def reference(A_x, A_wqkv, A_wo, B_x, B_w_gate, B_w_up, B_w_down):
    def _A_ref(x, wqkv, wo):
        B, S, D = x.shape
        H = 32; Dh = D // H
        qkv = (lambda x, *d: x.transpose(*d))((x @ wqkv).reshape(B, S, 3, H, Dh), 2, 0, 3, 1, 4)
        q, k, v = qkv[0], qkv[1], qkv[2]
        scale = Dh ** -0.5
        scores = jnp.einsum("bhqd,bhkd->bhqk", q, k) * scale
        p = _softmax(scores, axis=-1)
        o = jnp.einsum("bhqk,bhkd->bhqd", p, v)
        return (lambda x, *d: x.transpose(*d))(o, 0, 2, 1, 3).reshape(B, S, D) @ wo

    def _B_ref(x, w_gate, w_up, w_down):
        return (_gelu(x @ w_gate) * (x @ w_up)) @ w_down

    x = A_x
    h = x + _A_ref(_layernorm(x, axis=-1), A_wqkv, A_wo)
    h2 = h + _B_ref(_layernorm(h, axis=-1), B_w_gate, B_w_up, B_w_down)
    return h2
```

```python
import functools

import jax
import jax.numpy as jnp
from jax import lax
import jax.experimental.pallas as pl
import jax.experimental.pallas.tpu as pltpu

f32 = jnp.float32
bf16 = jnp.bfloat16
i32 = jnp.int32
i8 = jnp.int8

H = 32
DH = 16
TQ = 512
TB = 512
CK = 128
UNROLL = 4
LAG = 2
NSAMP = 32
EPS = 1e-5
LOG2E = 1.4426950408889634
RND = 12582912.0
C2 = 28.0
L_MAX = 2.0 ** 64


def _bits(x):
    return lax.bitcast_convert_type(x, i32)


def _flt(x):
    return lax.bitcast_convert_type(x, f32)


def _layernorm(x):
    mu = jnp.mean(x, axis=-1, keepdims=True)
    xc = x - mu
    var = jnp.mean(xc * xc, axis=-1, keepdims=True)
    return xc * lax.rsqrt(var + EPS)


def _exp_field(z):
    return jnp.clip(lax.shift_right_logical(_bits(z), 23), 1, 252)


def _inv_pow2(e):
    return _flt(lax.shift_left(253 - e, 23))


def _kernel(x_ref, wqkv_ref, wo_hbm, wg_hbm, wu_hbm, wd_hbm, o_ref,
            wo_ref, wg_ref, wu_ref, wd_ref, sem,
            wt_ref, kl_ref, ql_ref, vt_ref, eq_ref, ek_ref, ot_ref, bad_ref,
            *, S, D, F):
    step = pl.program_id(0)
    NB = S // TB
    NCB = TB // CK
    NC = S // CK
    G = D // 128

    def weight_copies():
        return [pltpu.make_async_copy(src, dst, sem.at[i])
                for i, (src, dst) in enumerate(
                    ((wo_hbm, wo_ref), (wg_hbm, wg_ref), (wu_hbm, wu_ref), (wd_hbm, wd_ref)))]

    @pl.when(step == 0)
    def _():
        for cp in weight_copies():
            cp.start()
        wt_ref[0:D, :] = wqkv_ref[:, 0:D].T
        wt_ref[D:2 * D, :] = wqkv_ref[:, 2 * D:3 * D].T

        head_of_lane = lax.broadcasted_iota(i32, (H, D), 1) // DH
        head_row = lax.broadcasted_iota(i32, (H, D), 0)
        own = head_of_lane == head_row
        lane = lax.broadcasted_iota(i32, (TB // 4, 128), 1)

        for tb in range(NB):
            rows = slice(tb * TB, (tb + 1) * TB)
            xn = _layernorm(x_ref[rows, :].astype(f32)).astype(bf16)

            k = jnp.dot(xn, wqkv_ref[:, D:2 * D], preferred_element_type=f32)
            kabs = jnp.max(jnp.abs(k), axis=0, keepdims=True)
            kmax = jnp.max(jnp.where(own, kabs, 0.0), axis=1, keepdims=True)
            ek = _exp_field(kmax * (1.0 / 127.25))
            ek_ref[tb] = jnp.broadcast_to(ek, (H, 128))
            ksc = jnp.max(jnp.where(own, _inv_pow2(ek), 0.0), axis=0, keepdims=True)
            ks = k * ksc
            yh = ks + RND
            yl = (ks - (yh - RND)) * C2 + RND
            kh = pltpu.bitcast(_bits(yh).astype(i8), i32)
            kl = pltpu.bitcast(_bits(yl).astype(i8), i32)
            for g in range(G):
                cur = [kh[:, g * 128:(g + 1) * 128]]
                for sh in (64, 32, 16):
                    low = (lane & sh) == 0
                    nxt = []
                    for a in cur:
                        r = pltpu.roll(a, sh, 1)
                        nxt.append(jnp.where(low, a, r))
                        nxt.append(jnp.where(low, r, a))
                    cur = nxt
                klg = kl[:, g * 128:(g + 1) * 128]
                for j in range(8):
                    out = jnp.where(lane // DH == j, klg, cur[j])
                    kl_ref[g * 8 + j, rows, :] = pltpu.bitcast(out, i8)

            qt = lax.dot_general(wt_ref[0:D, :], xn, (((1,), (1,)), ((), ())),
                                 preferred_element_type=f32)
            cq = DH ** -0.5 * LOG2E / 7.0
            for h in range(H):
                qh = qt[h * DH:(h + 1) * DH, :] * cq
                qmax = jnp.max(jnp.abs(qh), axis=0, keepdims=True)
                eq = _exp_field(qmax * (1.0 / 124.0))
                eq_ref[h, :, rows] = eq
                xq = qh * _inv_pow2(eq)
                yb = xq + RND
                yr = (xq - (yb - RND)) * 7.0 + yb
                ya = xq * (7.0 / C2) + RND
                bb = jnp.concatenate([_bits(yb), _bits(yb)], axis=0).astype(i8)
                pair = [_bits(ya), _bits(yr)] if h % 2 == 0 else [_bits(yr), _bits(ya)]
                ar = jnp.concatenate(pair, axis=0).astype(i8)
                for pslot in range(4):
                    ql_ref[h, pslot * 32:(pslot + 1) * 32, rows] = (
                        ar if pslot == (h % 8) // 2 else bb)

            vt = lax.dot_general(wt_ref[D:2 * D, :], xn, (((1,), (1,)), ((), ())),
                                 preferred_element_type=f32)
            vt_ref[:, rows] = vt.astype(bf16)

    qcols = pl.ds(pl.multiple_of(step * TQ, TQ), TQ)

    def magic(h, blk):
        ek = ek_ref[blk, pl.ds(h, 1), :]
        ek = jnp.concatenate([ek] * (TQ // 128), axis=1)
        x = jnp.clip(eq_ref[h, :, qcols] + ek - 102, 1, 254)
        return lax.shift_left(x, 23) | (1 << 22)

    def hrows(h):
        return pl.ds(pl.multiple_of(h * DH, DH), DH)

    bad_ref[...] = jnp.zeros_like(bad_ref)

    def fast_body(it, carry):
        items = [(u, c) for u in range(UNROLL) for c in range(NC)]
        ps = {}
        acc = [None] * UNROLL
        lsum = [None] * UNROLL
        off = [None] * UNROLL
        ab = {}
        for t in range(len(items) + LAG):
            if t < len(items):
                u, c = items[t]
                h = UNROLL * it + u
                blk = c // NCB
                s = jnp.dot(kl_ref[h, c * CK:(c + 1) * CK, :], ql_ref[h, :, qcols],
                            preferred_element_type=i32)
                if c % NCB == 0:
                    a = magic(h, blk)
                    if c == 0:
                        b = jnp.max(_flt(s[0:NSAMP] + a), axis=0, keepdims=True)
                        off[u] = b - _flt(a)
                    else:
                        b = _flt(a) + off[u]
                    ab[u] = (a, b)
                a, b = ab[u]
                p = jnp.exp2(_flt(s + a) - b)
                lc = jnp.sum(p.reshape(CK // 8, 8, TQ), axis=0)
                lsum[u] = lc if lsum[u] is None else lsum[u] + lc
                ps[t] = p.astype(bf16)
            if t >= LAG:
                u, c = items[t - LAG]
                h = UNROLL * it + u
                o = jnp.dot(vt_ref[hrows(h), c * CK:(c + 1) * CK], ps.pop(t - LAG),
                            preferred_element_type=f32)
                acc[u] = o if acc[u] is None else acc[u] + o
                if c == NC - 1:
                    l = jnp.sum(lsum[u], axis=0, keepdims=True)
                    o = acc[u] * (1.0 / l)
                    ok = jnp.logical_and(l <= L_MAX, jnp.abs(o) <= 3e38)
                    bad_ref[...] = jnp.maximum(bad_ref[...], jnp.where(ok, 0.0, 1.0))
                    ot_ref[hrows(h), :] = o.astype(bf16)
        return carry

    lax.fori_loop(0, H // UNROLL, fast_body, 0)

    @pl.when(jnp.max(bad_ref[...]) > 0.0)
    def _():
        def safe_body(h, carry):
            def scores(blk):
                a = magic(h, blk)
                s = jnp.dot(kl_ref[h, blk * TB:(blk + 1) * TB, :], ql_ref[h, :, qcols],
                            preferred_element_type=i32)
                return _flt(s + a) - _flt(a)

            m = None
            for blk in range(NB):
                mb = jnp.max(scores(blk), axis=0, keepdims=True)
                m = mb if m is None else jnp.maximum(m, mb)
            l = jnp.zeros((1, TQ), f32)
            acc = jnp.zeros((DH, TQ), f32)
            for blk in range(NB):
                p = jnp.exp2(scores(blk) - m)
                l = l + jnp.sum(p, axis=0, keepdims=True)
                acc = acc + jnp.dot(vt_ref[hrows(h), blk * TB:(blk + 1) * TB], p.astype(bf16),
                                    preferred_element_type=f32)
            ot_ref[hrows(h), :] = (acc * (1.0 / l)).astype(bf16)
            return carry

        lax.fori_loop(0, H, safe_body, 0)

    @pl.when(step == 0)
    def _():
        for cp in weight_copies():
            cp.wait()

    TM = 256
    for r in range(TQ // TM):
        attn = lax.dot_general(ot_ref[:, r * TM:(r + 1) * TM], wo_ref[...],
                               (((0,), (0,)), ((), ())), preferred_element_type=f32)
        xr = x_ref[pl.ds(pl.multiple_of(step * TQ + r * TM, TM), TM), :]
        hres = xr.astype(f32) + attn
        hn = _layernorm(hres).astype(bf16)
        gate = lax.dot_general(hn, wg_ref[...], (((1,), (1,)), ((), ())),
                               preferred_element_type=f32)
        up = lax.dot_general(hn, wu_ref[...], (((1,), (1,)), ((), ())),
                             preferred_element_type=f32)
        act = (jax.nn.gelu(gate, approximate=True) * up).astype(bf16)
        y = jnp.dot(act, wd_ref[...], preferred_element_type=f32)
        o_ref[r * TM:(r + 1) * TM, :] = (hres + y).astype(o_ref.dtype)


@jax.jit
def pallas_sequential_preLN__softmax_full_mha__geglu_ffn__prompt_kernel(
    A_x: jax.Array,
    A_wqkv: jax.Array,
    A_wo: jax.Array,
    B_x: jax.Array,
    B_w_gate: jax.Array,
    B_w_up: jax.Array,
    B_w_down: jax.Array,
):
    del B_x
    B, S, D = A_x.shape
    F = B_w_gate.shape[1]
    assert B == 1 and D == H * DH and S % TQ == 0 and S % TB == 0
    x = A_x.reshape(S, D)

    out = pl.pallas_call(
        functools.partial(_kernel, S=S, D=D, F=F),
        grid=(S // TQ,),
        in_specs=[
            pl.BlockSpec((S, D), lambda i: (0, 0)),
            pl.BlockSpec((D, 3 * D), lambda i: (0, 0)),
            pl.BlockSpec(memory_space=pl.ANY),
            pl.BlockSpec(memory_space=pl.ANY),
            pl.BlockSpec(memory_space=pl.ANY),
            pl.BlockSpec(memory_space=pl.ANY),
        ],
        out_specs=pl.BlockSpec((TQ, D), lambda i: (i, 0)),
        out_shape=jax.ShapeDtypeStruct((S, D), A_x.dtype),
        scratch_shapes=[
            pltpu.VMEM((D, D), bf16),
            pltpu.VMEM((F, D), bf16),
            pltpu.VMEM((F, D), bf16),
            pltpu.VMEM((F, D), bf16),
            pltpu.SemaphoreType.DMA((4,)),
            pltpu.VMEM((2 * D, D), bf16),
            pltpu.VMEM((H, S, 128), i8),
            pltpu.VMEM((H, 128, S), i8),
            pltpu.VMEM((D, S), bf16),
            pltpu.VMEM((H, 1, S), i32),
            pltpu.VMEM((S // TB, H, 128), i32),
            pltpu.VMEM((D, TQ), bf16),
            pltpu.VMEM((DH, TQ), f32),
        ],
        compiler_params=pltpu.CompilerParams(
            dimension_semantics=("arbitrary",),
            vmem_limit_bytes=100 * 1024 * 1024,
        ),
    )(x, A_wqkv, A_wo, B_w_gate.T, B_w_up.T, B_w_down)
    return out.reshape(B, S, D)
```

```python
import functools

import jax
import jax.numpy as jnp
from jax import lax
import jax.experimental.pallas as pl
import jax.experimental.pallas.tpu as pltpu

f32 = jnp.float32
bf16 = jnp.bfloat16
i32 = jnp.int32
i8 = jnp.int8

H = 32
DH = 16
TQ = 512
TB = 512
CK = 256
LAGH = 2
GROUPS = [2] * 8
UNROLL = 16
TM = 256
KSUB = 128
TSPAN = 6.0
PLOOP = True
EARLY_CUT = 1
EPS = 1e-5
LOG2E = 1.4426950408889634
RND = 12582912.0
C2 = 28.0
LIMIT = 2.0 ** 64
TINY = 2.0 ** -120
HUGE = 2.0 ** 120
EXP_MASK = 0x7F800000
NT = (((1,), (1,)), ((), ()))
TN = (((0,), (0,)), ((), ()))


def _bits(x):
    return lax.bitcast_convert_type(x, i32)


def _flt(x):
    return lax.bitcast_convert_type(x, f32)


def _layernorm(x):
    mu = jnp.mean(x, axis=-1, keepdims=True)
    xc = x - mu
    var = jnp.mean(xc * xc, axis=-1, keepdims=True)
    return xc * lax.rsqrt(var + EPS)


def _pow2_floor_bits(z):
    return _bits(jnp.minimum(jnp.maximum(z, TINY), HUGE)) & EXP_MASK


def _half_inv(pbits):
    return _flt((253 << 23) - pbits)


def _kernel(x_hbm, wqkv_hbm, wo_hbm, wg_hbm, wu_hbm, wd_hbm, o_ref,
            x_ref, wk_ref, wv_ref, wq_ref, wo_ref, wg_ref, wu_ref, wd_ref, sem,
            wt_ref, kl_ref, ql_ref, vt_ref, pq_ref, off_ref, pk_ref, ot_ref, chk_ref, xn_ref,
            *, S, D, F):
    step = pl.program_id(0)
    NB = S // TB
    NCB = TB // CK
    NC = S // CK
    G = D // 128

    def x_copy(tb):
        return pltpu.make_async_copy(x_hbm.at[tb * TB:(tb + 1) * TB, :],
                                     x_ref.at[tb * TB:(tb + 1) * TB, :], sem.at[tb])

    def w_copy(i):
        src, dst = ((wqkv_hbm.at[:, D:2 * D], wk_ref), (wqkv_hbm.at[:, 2 * D:3 * D], wv_ref),
                    (wqkv_hbm.at[:, 0:D], wq_ref), (wo_hbm, wo_ref), (wg_hbm, wg_ref),
                    (wu_hbm, wu_ref), (wd_hbm, wd_ref))[i]
        return pltpu.make_async_copy(src, dst, sem.at[NB + i])

    @pl.when(step == 0)
    @jax.named_scope("proj")
    def _():
        x_copy(0).start()
        w_copy(0).start()
        w_copy(1).start()
        w_copy(2).start()
        x_copy(1).start()
        x_copy(0).wait()

        own8 = (lax.broadcasted_iota(i32, (8, 128), 1) // DH) == lax.broadcasted_iota(i32, (8, 128), 0)
        own = (lax.broadcasted_iota(i32, (H, D), 1) // DH) == lax.broadcasted_iota(i32, (H, D), 0)
        lane = lax.broadcasted_iota(i32, (KSUB // 4, 128), 1)
        sc = DH ** -0.5 * LOG2E
        cq = sc / 7.0

        nsb = TB // KSUB

        def at(tb, off, size):
            start = tb * TB + off
            if isinstance(start, int):
                return slice(start, start + size)
            return pl.ds(pl.multiple_of(start, 128), size)

        def key_limbs(tb, k, vt, pieces, kscs):
            for idx in pieces:
                g, sb = idx // nsb, idx % nsb
                kg = k[:, g * 128:(g + 1) * 128]
                if g not in kscs:
                    kabs = jnp.max(jnp.abs(kg), axis=0, keepdims=True)
                    kmax = jnp.max(jnp.where(own8, kabs, 0.0), axis=1, keepdims=True)
                    pk = _pow2_floor_bits(kmax * (1.0 / 127.25))
                    pk_ref[tb, g * 8:(g + 1) * 8, :] = jnp.broadcast_to(
                        _flt(pk) * (1.5 * 2.0 ** 25), (8, 128))
                    kscs[g] = jnp.max(jnp.where(own8, _half_inv(pk), 0.0), axis=0, keepdims=True)
                ksc = kscs[g]
                tau = idx * TSPAN / (G * nsb)
                tile = int(tau)
                tr = int((tau - tile) * TB) // 8 * 8
                if tile < G - 1:
                    tie = k[tr:tr + 1, (tile + 1) * 128:(tile + 2) * 128]
                else:
                    tc = (tile - (G - 1)) * 128
                    tie = vt[tr:tr + 1, tc:tc + 128]
                kscg = jnp.minimum(ksc, jnp.maximum(ksc, tie))
                ks = kg[sb * KSUB:(sb + 1) * KSUB] * kscg
                yh = ks + RND
                yl = (ks - (yh - RND)) * C2 + RND
                kh = pltpu.bitcast(_bits(yh).astype(i8), i32)
                kl = pltpu.bitcast(_bits(yl).astype(i8), i32)
                cur = [kl] + [pltpu.roll(kh, DH * j, 1) for j in range(1, 8)]
                for bit in (1, 2, 4):
                    on = (lane & (DH * bit)) != 0
                    cur = [jnp.where(on, cur[(j + bit) % 8], cur[j]) for j in range(8)]
                for j in range(8):
                    kl_ref[g * 8 + (-j) % 8, at(tb, sb * KSUB, KSUB), :] = pltpu.bitcast(cur[j], i8)

        npieces = G * nsb
        nearly = len([i for i in range(npieces) if int(i * TSPAN / npieces) < G - 1]) - EARLY_CUT

        def norm(tb):
            return _layernorm(x_ref[at(tb, 0, TB), :].astype(f32)).astype(bf16)

        def kv_proj(tb, xn, mid=None):
            k = jnp.dot(xn, wk_ref[...], preferred_element_type=f32)
            kscs = {}
            key_limbs(tb, k, None, range(nearly), kscs)
            if mid is not None:
                mid(k)
            vt = lax.dot_general(wt_ref[0:D, :], xn, NT, preferred_element_type=f32)
            vt_ref[:, at(tb, 0, TB)] = vt.astype(bf16)
            key_limbs(tb, k, vt, range(nearly, npieces), kscs)

        def q_proj(tb, xn):
            qt = lax.dot_general(wt_ref[D:2 * D + H, :], xn, NT, preferred_element_type=f32)
            off_ref[:, at(tb, 0, TB)] = qt[D:D + H, :]
            for j in range(TB // 128):
                cols = at(tb, j * 128, 128)
                for h in range(H):
                    qh = qt[h * DH:(h + 1) * DH, j * 128:(j + 1) * 128]
                    qmax = jnp.max(jnp.abs(qh), axis=0, keepdims=True)
                    pq = _pow2_floor_bits(qmax * (cq / 124.0))
                    pq_ref[h:h + 1, cols] = _flt(pq)
                    xq = qh * (_half_inv(pq) * cq)
                    yb = xq + RND
                    yr = (xq - (yb - RND)) * 7.0 + yb
                    ya = xq * (7.0 / C2) + RND
                    bb = jnp.concatenate([_bits(yb), _bits(yb)], axis=0).astype(i8)
                    pair = [_bits(ya), _bits(yr)] if h % 2 == 0 else [_bits(yr), _bits(ya)]
                    ar = jnp.concatenate(pair, axis=0).astype(i8)
                    for pslot in range(4):
                        ql_ref[h, pslot * 32:(pslot + 1) * 32, cols] = (
                            ar if pslot == (h % 8) // 2 else bb)

        kd = []

        def mid(k):
            kbar = jnp.sum(k, axis=0, keepdims=True) * (sc / TB)
            kd.append(jnp.where(own, kbar, 0.0).astype(bf16))
            w_copy(1).wait()
            w_copy(2).wait()
            x_copy(1).wait()
            for j in range(2, NB):
                x_copy(j).start()
            for j in range(3, 7):
                w_copy(j).start()
            wt_ref[0:D, :] = wv_ref[...].T
            wt_ref[D:2 * D, :] = wq_ref[...].T

        xn = norm(0)
        w_copy(0).wait()
        kv_proj(0, xn, mid)
        wt_ref[2 * D:2 * D + H, :] = jnp.dot(
            kd[0], wt_ref[D:2 * D, :], preferred_element_type=f32).astype(bf16)
        q_proj(0, xn)
        xn = norm(1)
        kv_proj(1, xn)
        xn_ref[...] = xn
        for j in range(2, NB):
            x_copy(j).wait()

        def blk_body(tb, carry):
            q_proj(tb - 1, xn_ref[...])
            xn = norm(tb)
            kv_proj(tb, xn)
            xn_ref[...] = xn
            return carry

        if PLOOP:
            lax.fori_loop(2, NB, blk_body, 0)
        else:
            for tb in range(2, NB):
                blk_body(tb, 0)
        q_proj(NB - 1, xn_ref[...])

    qcols = pl.ds(pl.multiple_of(step * TQ, TQ), TQ)

    def magic(h, blk):
        pk = pk_ref[blk, pl.ds(h, 1), :]
        pk = jnp.concatenate([pk] * (TQ // 128), axis=1)
        c = pq_ref[pl.ds(h, 1), qcols] * pk
        return jnp.minimum(jnp.maximum(c, 1.5 * TINY), 1.5 * HUGE)

    def hrows(h):
        return pl.ds(pl.multiple_of(h * DH, DH), DH)

    chk_ref[...] = jnp.zeros_like(chk_ref)

    def fast_body(it, carry):
        starts = [sum(GROUPS[:i]) for i in range(len(GROUPS))]
        items = [(u, st, n) for u in range(UNROLL) for st, n in zip(starts, GROUPS)]
        NS = S // 128
        nsub = UNROLL * NS
        ps = {}
        acc = [None] * UNROLL
        lsum = [None] * UNROLL
        ab = {}
        done = 0
        issued = 0
        t = 0
        while done < nsub:
            if t < len(items):
                u, st, n = items[t]
                h = UNROLL * it + u
                s = jnp.dot(kl_ref[h, st * 128:(st + n) * 128, :], ql_ref[h, :, qcols],
                            preferred_element_type=i32)
                for r in range(n):
                    blk = (st + r) * 128 // TB
                    if (u, blk) not in ab:
                        cm = magic(h, blk)
                        ab[(u, blk)] = (_bits(cm), cm + off_ref[pl.ds(h, 1), qcols])
                    a, b = ab[(u, blk)]
                    p = jnp.exp2(_flt(s[r * 128:(r + 1) * 128] + a) - b)
                    lc = jnp.sum(p.reshape(16, 8, TQ), axis=0)
                    lsum[u] = lc if lsum[u] is None else lsum[u] + lc
                    ps[u * NS + st + r] = p.astype(bf16)
                issued += n
                upto = issued - (LAGH if LAGH > 0 else n)
            else:
                upto = nsub
            while done < upto:
                u, cc = done // NS, done % NS
                h = UNROLL * it + u
                o = jnp.dot(vt_ref[hrows(h), cc * 128:(cc + 1) * 128], ps.pop(done),
                            preferred_element_type=f32)
                acc[u] = o if acc[u] is None else o + acc[u]
                if cc == NS - 1:
                    l = jnp.sum(lsum[u], axis=0, keepdims=True)
                    r0 = pl.reciprocal(l, approx=True)
                    o = acc[u] * (r0 * (2.0 - l * r0))
                    big = jnp.maximum(jnp.maximum(l, r0 * 2.0 ** 40), jnp.abs(o[0:8] + o[8:16]))
                    chk_ref[...] = jnp.maximum(chk_ref[...], big)
                    ot_ref[hrows(h), :] = o.astype(bf16)
                done += 1
            t += 1
        return carry

    with jax.named_scope("attn"):
        lax.fori_loop(0, H // UNROLL, fast_body, 0)

    @pl.when(jnp.max(jnp.where(chk_ref[...] <= LIMIT, 0.0, 1.0)) > 0.0)
    def _():
        def safe_body(h, carry):
            def scores(blk):
                cm = magic(h, blk)
                s = jnp.dot(kl_ref[h, pl.ds(pl.multiple_of(blk * TB, TB), TB), :], ql_ref[h, :, qcols],
                            preferred_element_type=i32)
                return _flt(s + _bits(cm)) - cm

            def max_body(blk, m):
                return jnp.maximum(m, jnp.max(scores(blk), axis=0, keepdims=True))

            m = lax.fori_loop(0, NB, max_body, jnp.full((1, TQ), -jnp.inf, f32))

            def acc_body(blk, la):
                l, acc = la
                p = jnp.exp2(scores(blk) - m)
                l = l + jnp.sum(p, axis=0, keepdims=True)
                acc = acc + jnp.dot(vt_ref[hrows(h), pl.ds(pl.multiple_of(blk * TB, TB), TB)],
                                    p.astype(bf16), preferred_element_type=f32)
                return l, acc

            l, acc = lax.fori_loop(0, NB, acc_body,
                                   (jnp.zeros((1, TQ), f32), jnp.zeros((DH, TQ), f32)))
            ot_ref[hrows(h), :] = (acc * (1.0 / l)).astype(bf16)
            return carry

        lax.fori_loop(0, H, safe_body, 0)

    @pl.when(step == 0)
    def _():
        for j in range(3, 7):
            w_copy(j).wait()

    with jax.named_scope("ffn"):
        hres, hn = [], []
        for r in range(TQ // TM):
            attn = lax.dot_general(ot_ref[:, r * TM:(r + 1) * TM], wo_ref[...], TN,
                                   preferred_element_type=f32)
            xr = x_ref[pl.ds(pl.multiple_of(step * TQ + r * TM, TM), TM), :]
            hres.append(xr.astype(f32) + attn)
            hn.append(_layernorm(hres[r]).astype(bf16))
        for r in range(TQ // TM):
            gate = lax.dot_general(hn[r], wg_ref[...], NT, preferred_element_type=f32)
            up = lax.dot_general(hn[r], wu_ref[...], NT, preferred_element_type=f32)
            act = (jax.nn.gelu(gate, approximate=True) * up).astype(bf16)
            y = jnp.dot(act, wd_ref[...], preferred_element_type=f32)
            o_ref[r * TM:(r + 1) * TM, :] = (hres[r] + y).astype(o_ref.dtype)


@jax.jit
def pallas_sequential_preLN__softmax_full_mha__geglu_ffn__prompt_kernel(
    A_x, A_wqkv, A_wo, B_x, B_w_gate, B_w_up, B_w_down,
):
    del B_x
    B, S, D = A_x.shape
    F = B_w_gate.shape[1]
    x = A_x.reshape(S, D)

    out = pl.pallas_call(
        functools.partial(_kernel, S=S, D=D, F=F),
        grid=(S // TQ,),
        in_specs=[pl.BlockSpec(memory_space=pl.ANY)] * 6,
        out_specs=pl.BlockSpec((TQ, D), lambda i: (i, 0)),
        out_shape=jax.ShapeDtypeStruct((S, D), A_x.dtype),
        scratch_shapes=[
            pltpu.VMEM((S, D), bf16),
            pltpu.VMEM((D, D), bf16),
            pltpu.VMEM((D, D), bf16),
            pltpu.VMEM((D, D), bf16),
            pltpu.VMEM((D, D), bf16),
            pltpu.VMEM((F, D), bf16),
            pltpu.VMEM((F, D), bf16),
            pltpu.VMEM((F, D), bf16),
            pltpu.SemaphoreType.DMA((S // TB + 7,)),
            pltpu.VMEM((2 * D + H, D), bf16),
            pltpu.VMEM((H, S, 128), i8),
            pltpu.VMEM((H, 128, S), i8),
            pltpu.VMEM((D, S), bf16),
            pltpu.VMEM((H, S), f32),
            pltpu.VMEM((H, S), f32),
            pltpu.VMEM((S // TB, H, 128), f32),
            pltpu.VMEM((D, TQ), bf16),
            pltpu.VMEM((8, TQ), f32),
            pltpu.VMEM((TB, D), bf16),
        ],
        compiler_params=pltpu.CompilerParams(
            dimension_semantics=("arbitrary",),
            vmem_limit_bytes=100 * 1024 * 1024,
        ),
    )(x, A_wqkv, A_wo, B_w_gate.T, B_w_up.T, B_w_down)
    return out.reshape(B, S, D)
```

```python
import functools
import math

import jax
import jax.numpy as jnp
from jax import lax
import jax.experimental.pallas as pl
import jax.experimental.pallas.tpu as pltpu

f32 = jnp.float32
bf16 = jnp.bfloat16
i32 = jnp.int32
i8 = jnp.int8

H = 32
DH = 16
TQ = 512
TB = 512
UNROLL = 16
GRP = 2
ORD = ((2, 3, 0, 1), (0, 1, 2, 3))
WSPLIT = 128
TT = 128
KSUB = 32
K1 = 3
V1 = 2
TSPAN = 6.0
EARLY = 0.3
LN_FIRST = tuple(6.1 + i * 0.15 for i in range(32))
LN_LOOP = tuple(0.05 + i * 0.225 for i in range(32))

EPS = 1e-5
LOG2E = 1.4426950408889634
RND = 12582912.0
C2 = 28.0
SHIFT = 32.0
LIMIT = 2.0 ** 100
TINY = 2.0 ** -120
HUGE = 2.0 ** 120
EXP_MASK = 0x7F800000
NT = (((1,), (1,)), ((), ()))
TN = (((0,), (0,)), ((), ()))


def _bits(x):
    return lax.bitcast_convert_type(x, i32)


def _flt(x):
    return lax.bitcast_convert_type(x, f32)


def _normalize(x, axis):
    mu = jnp.mean(x, axis=axis, keepdims=True)
    xc = x - mu
    var = jnp.mean(xc * xc, axis=axis, keepdims=True)
    return xc * lax.rsqrt(var + EPS)


def _pow2_floor_bits(z):
    return _bits(jnp.minimum(jnp.maximum(z, TINY), HUGE)) & EXP_MASK


def _half_inv(pbits):
    return _flt((253 << 23) - pbits)


def _after(x, tie):
    return jnp.minimum(x, jnp.maximum(x, tie))


def _split(arr):
    return [arr[:, j * 128:(j + 1) * 128] for j in range(arr.shape[1] // 128)]


def _pick(tiles, pos):
    tile = int(pos)
    row = int((pos - tile) * TB) // 8 * 8
    return tiles[tile][row:row + 1, :]


def _kernel(x_hbm, wqkv_hbm, wo_hbm, wg_hbm, wu_hbm, wd_hbm, o_hbm,
            x_ref, wkv_ref, wq_ref, wo_ref, wg_ref, wu_ref, wd_ref, sem,
            wt_ref, wot_ref, xn_ref, kl_ref, ql_ref, vt_ref, pq_ref, off_ref, pk_ref,
            ot_ref, ap_ref, of_ref, chk_ref, o_ref, *, S, D):
    step = pl.program_id(0)
    NB = S // TB
    NS = S // 128
    G = D // 128

    def at(tb, off, size):
        start = tb * TB + off
        if isinstance(start, int):
            return slice(start, start + size)
        return pl.ds(pl.multiple_of(start, math.gcd(TB, off)), size)

    def x_copy(tb, s):
        return pltpu.make_async_copy(x_hbm.at[at(tb, 0, TB), :], x_ref.at[at(tb, 0, TB), :],
                                     sem.at[s])

    ca = K1 * 128
    wk_copy = pltpu.make_async_copy(wqkv_hbm.at[:, D:D + ca], wkv_ref.at[:, 0:ca], sem.at[1])
    wv_copy = pltpu.make_async_copy(wqkv_hbm.at[:, D + ca:3 * D], wkv_ref.at[:, ca:2 * D], sem.at[2])
    wq_copy = pltpu.make_async_copy(wqkv_hbm.at[:, 0:D], wq_ref, sem.at[3])
    wo_copy = pltpu.make_async_copy(wo_hbm, wo_ref, sem.at[4])
    ffn_copies = [pltpu.make_async_copy(src, dst, sem.at[2])
                  for src, dst in ((wg_hbm, wg_ref), (wu_hbm, wu_ref), (wd_hbm, wd_ref))]

    @pl.when(step == 0)
    def _():
        x_copy(0, 0).start()
        wk_copy.start()
        wv_copy.start()
        wq_copy.start()
        x_copy(1, 3).start()
        wo_copy.start()
        x_copy(0, 0).wait()

        own8 = (lax.broadcasted_iota(i32, (8, 128), 1) // DH) == lax.broadcasted_iota(i32, (8, 128), 0)
        own = (lax.broadcasted_iota(i32, (H, D), 1) // DH) == lax.broadcasted_iota(i32, (H, D), 0)
        lane = lax.broadcasted_iota(i32, (KSUB // 4, 128), 1)
        sc = DH ** -0.5 * LOG2E
        cq = sc / 7.0
        nsb = TB // KSUB
        npieces = G * nsb

        def key_limbs(tb, tiles, pieces, kscs):
            for idx in pieces:
                g, sb = idx // nsb, idx % nsb
                if g not in kscs:
                    kabs = jnp.max(jnp.abs(tiles[g]), axis=0, keepdims=True)
                    kmax = jnp.max(jnp.where(own8, kabs, 0.0), axis=1, keepdims=True)
                    pk = _pow2_floor_bits(kmax * (1.0 / 127.25))
                    pk_ref[tb, g * 8:(g + 1) * 8, :] = jnp.broadcast_to(
                        _flt(pk) * (1.5 * 2.0 ** 25), (8, 128))
                    kscs[g] = jnp.max(jnp.where(own8, _half_inv(pk), 0.0), axis=0, keepdims=True)
                ksc = _after(kscs[g], _pick(tiles, 1.0 + idx * TSPAN / npieces))
                ks = tiles[g][sb * KSUB:(sb + 1) * KSUB] * ksc
                yh = ks + RND
                yl = (ks - (yh - RND)) * C2 + RND
                kh = pltpu.bitcast(_bits(yh).astype(i8), i32)
                kl = pltpu.bitcast(_bits(yl).astype(i8), i32)
                cur = [kl] + [pltpu.roll(kh, DH * j, 1) for j in range(1, 8)]
                for bit in (1, 2, 4):
                    on = (lane & (DH * bit)) != 0
                    cur = [jnp.where(on, cur[(j + bit) % 8], cur[j]) for j in range(8)]
                for j in range(8):
                    kl_ref[g * 8 + (-j) % 8, at(tb, sb * KSUB, KSUB), :] = pltpu.bitcast(cur[j], i8)

        def ready(ntiles):
            return len([i for i in range(npieces) if 1.0 + i * TSPAN / npieces < ntiles - EARLY])

        def norm_paced(tb, ties):
            rs = TB // len(ties)
            for i, tie in enumerate(ties):
                one = jnp.concatenate([_after(jnp.ones((1, 128), f32), tie)] * G, axis=1)
                xf = x_ref[at(tb, i * rs, rs), :].astype(f32) * one
                xn_ref[i * rs:(i + 1) * rs, :] = _normalize(xf, -1).astype(bf16)

        def k_tiles(xn, lo, hi):
            return _split(jnp.dot(xn, wkv_ref[:, lo * 128:hi * 128], preferred_element_type=f32))

        def v_tiles(tb, xn, lo, hi):
            vt = lax.dot_general(wt_ref[0:D, :], xn[lo * 128:hi * 128], NT,
                                 preferred_element_type=f32)
            vt_ref[:, at(tb, lo * 128, (hi - lo) * 128)] = vt.astype(bf16)
            return _split(vt)

        def q_proj(tb, xn):
            qt = lax.dot_general(wt_ref[D:2 * D + H, :], xn, NT, preferred_element_type=f32)
            off_ref[:, at(tb, 0, TB)] = qt[D:D + H, :] + SHIFT
            for j in range(TB // 128):
                cols = at(tb, j * 128, 128)
                for h in range(H):
                    qh = qt[h * DH:(h + 1) * DH, j * 128:(j + 1) * 128]
                    qmax = jnp.max(jnp.abs(qh), axis=0, keepdims=True)
                    pq = _pow2_floor_bits(qmax * (cq / 124.0))
                    pq_ref[h:h + 1, cols] = _flt(pq)
                    xq = qh * (_half_inv(pq) * cq)
                    yb = xq + RND
                    yr = (xq - (yb - RND)) * 7.0 + yb
                    ya = xq * (7.0 / C2) + RND
                    bb = jnp.concatenate([_bits(yb), _bits(yb)], axis=0).astype(i8)
                    pair = [_bits(ya), _bits(yr)] if h % 2 == 0 else [_bits(yr), _bits(ya)]
                    ar = jnp.concatenate(pair, axis=0).astype(i8)
                    for ps in range(4):
                        ql_ref[h, ps * 32:(ps + 1) * 32, cols] = ar if ps == (h % 8) // 2 else bb
            return _split(qt)

        xn = _normalize(x_ref[0:TB, :].astype(f32), -1).astype(bf16)
        wk_copy.wait()
        kscs = {}
        tiles = k_tiles(xn, 0, K1)
        n1 = ready(K1)
        key_limbs(0, tiles, range(n1), kscs)

        wv_copy.wait()
        for j in range(2, NB):
            x_copy(j, j - 2).start()
        for cp in ffn_copies:
            cp.start()
        wt_ref[0:D, :] = wkv_ref[:, D:2 * D].T
        tiles += k_tiles(xn, K1, G)
        kbar = jnp.concatenate([jnp.sum(t, axis=0, keepdims=True) for t in tiles], axis=1)
        kdiag = jnp.where(own, kbar * (sc / TB), 0.0).astype(bf16)
        tiles += v_tiles(0, xn, 0, V1)
        n2 = ready(G + V1)
        key_limbs(0, tiles, range(n1, n2), kscs)

        wq_copy.wait()
        x_copy(1, 3).wait()
        wt_ref[D:2 * D, :] = wq_ref[...].T
        tiles += v_tiles(0, xn, V1, G)
        key_limbs(0, tiles, range(n2, npieces), kscs)
        wt_ref[2 * D:2 * D + H, :] = jnp.dot(
            kdiag, wt_ref[D:2 * D, :], preferred_element_type=f32).astype(bf16)
        tiles += q_proj(0, xn)
        norm_paced(1, [_pick(tiles, p) for p in LN_FIRST])
        wo_copy.wait()

        def blk_body(tb, carry):
            @pl.when(tb + 1 < NB)
            def _():
                x_copy(tb + 1, tb - 1).wait()

            for g in range(2):
                rows = pl.ds(pl.multiple_of((tb - 1 + g) * 128, 128), 128)
                wot_ref[tb - 1 + g] = wo_ref[rows, :].T
            xn = xn_ref[...]
            q_proj(tb, xn)
            tiles = k_tiles(xn, 0, G) + v_tiles(tb, xn, 0, G)
            key_limbs(tb, tiles, range(npieces), {})
            norm_paced(jnp.minimum(tb + 1, NB - 1), [_pick(tiles, p) for p in LN_LOOP])
            return carry

        lax.fori_loop(1, NB, blk_body, 0)

    qcols = pl.ds(pl.multiple_of(step * TQ, TQ), TQ)

    def magic(h, blk):
        pk = jnp.concatenate([pk_ref[blk, pl.ds(h, 1), :]] * (TQ // 128), axis=1)
        c = pq_ref[pl.ds(h, 1), qcols] * pk
        return jnp.minimum(jnp.maximum(c, 1.5 * TINY), 1.5 * HUGE)

    def hrows(h):
        return pl.ds(pl.multiple_of(h * DH, DH), DH)

    def fast_body(it, bad):
        ps = {}
        acc = [None] * UNROLL
        lsum = [None] * UNROLL
        first = []

        def wo_part(lo, hi):
            ap_ref[it, lo:hi, :] = jnp.dot(wot_ref[2 * it, lo:hi, :], jnp.concatenate(first, axis=0),
                                           preferred_element_type=f32)

        def qk(u, st):
            h = UNROLL * it + u
            lhs = jnp.concatenate(
                [kl_ref[h, (st + r) * 128 + q * 32:(st + r) * 128 + (q + 1) * 32, :]
                 for r in range(GRP) for q in ORD[r]], axis=0)
            s = jnp.dot(lhs, ql_ref[h, :, qcols], preferred_element_type=i32)
            if st * 128 % TB == 0:
                c = magic(h, st * 128 // TB)
                ps["ab"] = (_bits(c), c + off_ref[pl.ds(h, 1), qcols])
            a, b = ps["ab"]
            for r in range(GRP):
                p = jnp.exp2(_flt(s[r * 128:(r + 1) * 128] + a) - b)
                lc = jnp.sum(p.reshape(16, 8, TQ), axis=0)
                lsum[u] = lc if lsum[u] is None else lsum[u] + lc
                p = jnp.concatenate([p[ORD[r].index(q) * 32:(ORD[r].index(q) + 1) * 32]
                                     for q in range(4)], axis=0)
                ps[(u, st + r)] = p.astype(bf16)

        def pv(u, st):
            h = UNROLL * it + u
            for c in range(st, st + GRP):
                o = jnp.dot(vt_ref[hrows(h), c * 128:(c + 1) * 128], ps.pop((u, c)),
                            preferred_element_type=f32)
                acc[u] = o if acc[u] is None else o + acc[u]
            if st + GRP == NS:
                l = jnp.sum(lsum[u], axis=0, keepdims=True)
                r0 = pl.reciprocal(l, approx=True)
                o = acc[u] * (r0 * (2.0 - l * r0))
                big = jnp.maximum(jnp.maximum(l, r0 * 2.0 ** 40), jnp.abs(o[0:8] + o[8:16]))
                chk_ref[...] = big if u == 0 else jnp.maximum(chk_ref[...], big)
                if u < 8:
                    first.append(o.astype(bf16))
                else:
                    ot_ref[hrows(8 * it + u - 8), :] = o.astype(bf16)

        items = [(u, st) for u in range(UNROLL) for st in range(0, NS, GRP)]
        for t, item in enumerate(items):
            qk(*item)
            if t > 0:
                pv(*items[t - 1])
        wo_part(0, WSPLIT)
        pv(*items[-1])
        wo_part(WSPLIT, D)
        return jnp.maximum(bad, jnp.max(jnp.where(chk_ref[...] <= LIMIT, 0.0, 1.0)))

    bad = lax.fori_loop(0, H // UNROLL, fast_body, jnp.float32(0.0))

    @pl.when(bad > 0.0)
    def _():
        def safe_body(h, carry):
            def scores(blk):
                c = magic(h, blk)
                s = jnp.dot(kl_ref[h, at(blk, 0, TB), :], ql_ref[h, :, qcols],
                            preferred_element_type=i32)
                return _flt(s + _bits(c)) - c

            def max_body(blk, m):
                return jnp.maximum(m, jnp.max(scores(blk), axis=0, keepdims=True))

            m = lax.fori_loop(0, NB, max_body, jnp.full((1, TQ), -jnp.inf, f32))

            def acc_body(blk, la):
                p = jnp.exp2(scores(blk) - m)
                o = jnp.dot(vt_ref[hrows(h), at(blk, 0, TB)], p.astype(bf16),
                            preferred_element_type=f32)
                return la[0] + jnp.sum(p, axis=0, keepdims=True), la[1] + o

            l, acc = lax.fori_loop(0, NB, acc_body,
                                   (jnp.zeros((1, TQ), f32), jnp.zeros((DH, TQ), f32)))
            of_ref[hrows(h), :] = (acc * (1.0 / l)).astype(bf16)
            return carry

        lax.fori_loop(0, H, safe_body, 0)
        for it in range(2):
            ap_ref[it] = jnp.dot(wot_ref[2 * it], of_ref[256 * it:256 * it + 128, :],
                                 preferred_element_type=f32)
            ot_ref[128 * it:128 * (it + 1), :] = of_ref[256 * it + 128:256 * (it + 1), :]

    @pl.when(step == 0)
    def _():
        for cp in ffn_copies:
            cp.wait()

    NJ = TQ // TT
    wdt = wd_ref[...].T
    wodd = jnp.concatenate([wot_ref[1], wot_ref[3]], axis=1)
    ht, hnt, acts = [], [], []

    def trows(j):
        return pl.ds(pl.multiple_of(step * TQ + j * TT, TT), TT)

    for j in range(NJ):
        cs = slice(j * TT, (j + 1) * TT)
        attn = jnp.dot(wodd, ot_ref[:, cs], preferred_element_type=f32)
        attn = attn + (ap_ref[0, :, cs] + ap_ref[1, :, cs])
        ht.append(x_ref[trows(j), :].T.astype(f32) + attn)
        hnt.append(_normalize(ht[j], 0).astype(bf16))

    def down(j):
        if j == NJ - 1:
            y = lax.dot_general(acts[j], wd_ref[...], TN, preferred_element_type=f32)
            o_ref[trows(j), :] = (ht[j].T + y).astype(o_ref.dtype)
        else:
            y = jnp.dot(wdt, acts[j], preferred_element_type=f32)
            o_ref[trows(j), :] = (ht[j] + y).astype(o_ref.dtype).T
        pltpu.make_async_copy(o_ref.at[trows(j), :], o_hbm.at[trows(j), :], sem.at[3]).start()

    for j in range(NJ):
        gate = jnp.dot(wg_ref[...], hnt[j], preferred_element_type=f32)
        up = jnp.dot(wu_ref[...], hnt[j], preferred_element_type=f32)
        acts.append((jax.nn.gelu(gate, approximate=True) * up).astype(bf16))
        if j > 0:
            down(j - 1)
    down(NJ - 1)

    @pl.when(step == pl.num_programs(0) - 1)
    def _():
        pltpu.make_async_copy(o_ref, o_hbm, sem.at[3]).wait()


@jax.jit
def pallas_sequential_preLN__softmax_full_mha__geglu_ffn__prompt_kernel(
    A_x: jax.Array,
    A_wqkv: jax.Array,
    A_wo: jax.Array,
    B_x: jax.Array,
    B_w_gate: jax.Array,
    B_w_up: jax.Array,
    B_w_down: jax.Array,
):
    del B_x
    B, S, D = A_x.shape
    F = B_w_gate.shape[1]
    assert B == 1 and D == H * DH == 512 and S == 4 * TB and H == 2 * UNROLL

    out = pl.pallas_call(
        functools.partial(_kernel, S=S, D=D),
        grid=(S // TQ,),
        in_specs=[pl.BlockSpec(memory_space=pl.ANY)] * 6,
        out_specs=pl.BlockSpec(memory_space=pl.ANY),
        out_shape=jax.ShapeDtypeStruct((S, D), A_x.dtype),
        scratch_shapes=[
            pltpu.VMEM((S, D), bf16),
            pltpu.VMEM((D, 2 * D), bf16),
            pltpu.VMEM((D, D), bf16),
            pltpu.VMEM((D, D), bf16),
            pltpu.VMEM((F, D), bf16),
            pltpu.VMEM((F, D), bf16),
            pltpu.VMEM((F, D), bf16),
            pltpu.SemaphoreType.DMA((5,)),
            pltpu.VMEM((2 * D + H, D), bf16),
            pltpu.VMEM((D // 128, D, 128), bf16),
            pltpu.VMEM((TB, D), bf16),
            pltpu.VMEM((H, S, 128), i8),
            pltpu.VMEM((H, 128, S), i8),
            pltpu.VMEM((D, S), bf16),
            pltpu.VMEM((H, S), f32),
            pltpu.VMEM((H, S), f32),
            pltpu.VMEM((S // TB, H, 128), f32),
            pltpu.VMEM((D // 2, TQ), bf16),
            pltpu.VMEM((2, D, TQ), f32),
            pltpu.VMEM((D, TQ), bf16),
            pltpu.VMEM((8, TQ), f32),
            pltpu.VMEM((S, D), A_x.dtype),
        ],
        compiler_params=pltpu.CompilerParams(
            dimension_semantics=("arbitrary",),
            vmem_limit_bytes=100 * 1024 * 1024,
        ),
    )(A_x.reshape(S, D), A_wqkv, A_wo, B_w_gate.T, B_w_up.T, B_w_down)
    return out.reshape(B, S, D)
```

```python
import functools
import math

import jax
import jax.numpy as jnp
from jax import lax
import jax.experimental.pallas as pl
import jax.experimental.pallas.tpu as pltpu

f32 = jnp.float32
bf16 = jnp.bfloat16
i32 = jnp.int32
i8 = jnp.int8

H = 32
DH = 16
TQ = 512
TB = 512
UNROLL = 16
GRP = 2
ORD = ((1, 3, 2, 0), (2, 0, 1, 3))
WSPLIT = 144
TT = 128
KSUB = 32
K1 = 3
V1 = 2
TSPAN = 6.0
EARLY = 0.3
LN_FIRST = tuple(6.1 + i * 0.15 for i in range(32))
LN_LOOP = tuple(0.05 + i * 0.225 for i in range(32))

EPS = 1e-5
LOG2E = 1.4426950408889634
RND = 12582912.0
C2 = 28.0
MAX_BAL = 2.0 ** 12
SHIFT = 32.0
LIMIT = 2.0 ** 100
TINY = 2.0 ** -120
HUGE = 2.0 ** 120
EXP_MASK = 0x7F800000
NT = (((1,), (1,)), ((), ()))
TN = (((0,), (0,)), ((), ()))


def _bits(x):
    return lax.bitcast_convert_type(x, i32)


def _flt(x):
    return lax.bitcast_convert_type(x, f32)


def _normalize(x, axis):
    mu = jnp.mean(x, axis=axis, keepdims=True)
    xc = x - mu
    var = jnp.mean(xc * xc, axis=axis, keepdims=True)
    return xc * lax.rsqrt(var + EPS)


def _pow2_floor_bits(z):
    return _bits(jnp.minimum(jnp.maximum(z, TINY), HUGE)) & EXP_MASK


def _half_inv(pbits):
    return _flt((253 << 23) - pbits)


def _after(x, tie):
    return jnp.minimum(x, jnp.maximum(x, tie))


def _split(arr):
    return [arr[:, j * 128:(j + 1) * 128] for j in range(arr.shape[1] // 128)]


def _pick(tiles, pos):
    tile = int(pos)
    row = int((pos - tile) * TB) // 8 * 8
    return tiles[tile][row:row + 1, :]


def _kernel(x_hbm, wqkv_hbm, wo_hbm, wg_hbm, wu_hbm, wd_hbm, o_hbm,
            x_ref, wkv_ref, wq_ref, wo_ref, wg_ref, wu_ref, wd_ref, sem,
            wt_ref, wot_ref, xn_ref, kl_ref, ql_ref, vt_ref, pq_ref, off_ref, pk_ref, bal_ref,
            ot_ref, ap_ref, of_ref, chk_ref, o_ref, *, S, D):
    step = pl.program_id(0)
    NB = S // TB
    NS = S // 128
    G = D // 128

    def at(tb, off, size):
        start = tb * TB + off
        if isinstance(start, int):
            return slice(start, start + size)
        return pl.ds(pl.multiple_of(start, math.gcd(TB, off)), size)

    def x_copy(tb, s):
        return pltpu.make_async_copy(x_hbm.at[at(tb, 0, TB), :], x_ref.at[at(tb, 0, TB), :],
                                     sem.at[s])

    ca = K1 * 128
    wk_copy = pltpu.make_async_copy(wqkv_hbm.at[:, D:D + ca], wkv_ref.at[:, 0:ca], sem.at[1])
    wv_copy = pltpu.make_async_copy(wqkv_hbm.at[:, D + ca:3 * D], wkv_ref.at[:, ca:2 * D], sem.at[2])
    wq_copy = pltpu.make_async_copy(wqkv_hbm.at[:, 0:D], wq_ref, sem.at[3])
    wo_copy = pltpu.make_async_copy(wo_hbm, wo_ref, sem.at[4])
    ffn_copies = [pltpu.make_async_copy(src, dst, sem.at[2])
                  for src, dst in ((wg_hbm, wg_ref), (wu_hbm, wu_ref), (wd_hbm, wd_ref))]

    @pl.when(step == 0)
    def _():
        x_copy(0, 0).start()
        wk_copy.start()
        wv_copy.start()
        wq_copy.start()
        x_copy(1, 3).start()
        wo_copy.start()
        x_copy(0, 0).wait()

        own8 = (lax.broadcasted_iota(i32, (8, 128), 1) // DH) == lax.broadcasted_iota(i32, (8, 128), 0)
        own = (lax.broadcasted_iota(i32, (H, D), 1) // DH) == lax.broadcasted_iota(i32, (H, D), 0)
        lane = lax.broadcasted_iota(i32, (KSUB // 4, 128), 1)
        sc = DH ** -0.5 * LOG2E
        cq = sc / 7.0
        nsb = TB // KSUB
        npieces = G * nsb

        def key_limbs(tb, tiles, pieces, kscs):
            for idx in pieces:
                g, sb = idx // nsb, idx % nsb
                if g not in kscs:
                    gl = slice(g * 128, (g + 1) * 128)
                    kabs = jnp.max(jnp.abs(tiles[g]), axis=0, keepdims=True)
                    if isinstance(tb, int):
                        wabs = jnp.sum(jnp.abs(wkv_ref[:, gl].astype(f32)), axis=0, keepdims=True)
                        top = jnp.max(jnp.where(own8, wabs, 0.0), axis=1, keepdims=True)
                        top = jnp.max(jnp.where(own8, top, 0.0), axis=0, keepdims=True)
                        ratio = jnp.clip(top / jnp.maximum(wabs, TINY), 1.0, MAX_BAL)
                        pb = _bits(ratio) & EXP_MASK
                        bal_ref[0:1, gl] = _flt(pb)
                        bal_ref[1:2, gl] = _flt((254 << 23) - pb)
                    bal = bal_ref[0:1, gl]
                    kmax = jnp.max(jnp.where(own8, kabs * bal, 0.0), axis=1, keepdims=True)
                    pk = _pow2_floor_bits(kmax * (1.0 / 127.25))
                    pk_ref[tb, g * 8:(g + 1) * 8, :] = jnp.broadcast_to(
                        _flt(pk) * (1.5 * 2.0 ** 25), (8, 128))
                    kscs[g] = bal * jnp.max(jnp.where(own8, _half_inv(pk), 0.0), axis=0, keepdims=True)
                ksc = _after(kscs[g], _pick(tiles, 1.0 + idx * TSPAN / npieces))
                ks = tiles[g][sb * KSUB:(sb + 1) * KSUB] * ksc
                fh = jnp.floor(ks + 0.5)
                yh = fh + RND
                yl = (ks - fh) * C2 + RND
                kh = pltpu.bitcast(_bits(yh).astype(i8), i32)
                kl = pltpu.bitcast(_bits(yl).astype(i8), i32)
                cur = [kl] + [pltpu.roll(kh, DH * j, 1) for j in range(1, 8)]
                for bit in (1, 2, 4):
                    on = (lane & (DH * bit)) != 0
                    cur = [jnp.where(on, cur[(j + bit) % 8], cur[j]) for j in range(8)]
                for j in range(8):
                    kl_ref[g * 8 + (-j) % 8, at(tb, sb * KSUB, KSUB), :] = pltpu.bitcast(cur[j], i8)

        def ready(ntiles):
            return len([i for i in range(npieces) if 1.0 + i * TSPAN / npieces < ntiles - EARLY])

        def norm_paced(tb, ties):
            rs = TB // len(ties)
            for i, tie in enumerate(ties):
                one = jnp.concatenate([_after(jnp.ones((1, 128), f32), tie)] * G, axis=1)
                xf = x_ref[at(tb, i * rs, rs), :].astype(f32) * one
                xn_ref[i * rs:(i + 1) * rs, :] = _normalize(xf, -1).astype(bf16)

        def k_tiles(xn, lo, hi):
            return _split(jnp.dot(xn, wkv_ref[:, lo * 128:hi * 128], preferred_element_type=f32))

        def v_tiles(tb, xn, lo, hi):
            vt = lax.dot_general(wt_ref[0:D, :], xn[lo * 128:hi * 128], NT,
                                 preferred_element_type=f32)
            vt_ref[:, at(tb, lo * 128, (hi - lo) * 128)] = vt.astype(bf16)
            return _split(vt)

        def q_proj(tb, xn):
            qt = lax.dot_general(wt_ref[D:2 * D + H, :], xn, NT, preferred_element_type=f32)
            off_ref[:, at(tb, 0, TB)] = qt[D:D + H, :] + SHIFT
            for j in range(TB // 128):
                cols = at(tb, j * 128, 128)
                for h in range(H):
                    qh = qt[h * DH:(h + 1) * DH, j * 128:(j + 1) * 128]
                    qmax = jnp.max(jnp.abs(qh), axis=0, keepdims=True)
                    pq = _pow2_floor_bits(qmax * (cq / 124.0))
                    pq_ref[h:h + 1, cols] = _flt(pq)
                    xq = qh * (_half_inv(pq) * cq)
                    fb = jnp.floor(xq + 0.5)
                    yb = fb + RND
                    yr = (xq - fb) * 7.0 + yb
                    ya = xq * (7.0 / C2) + RND
                    bb = jnp.concatenate([_bits(yb), _bits(yb)], axis=0).astype(i8)
                    pair = [_bits(ya), _bits(yr)] if h % 2 == 0 else [_bits(yr), _bits(ya)]
                    ar = jnp.concatenate(pair, axis=0).astype(i8)
                    for ps in range(4):
                        ql_ref[h, ps * 32:(ps + 1) * 32, cols] = ar if ps == (h % 8) // 2 else bb
            return _split(qt)

        xn = _normalize(x_ref[0:TB, :].astype(f32), -1).astype(bf16)
        wk_copy.wait()
        kscs = {}
        tiles = k_tiles(xn, 0, K1)
        n1 = ready(K1)
        key_limbs(0, tiles, range(n1), kscs)

        wv_copy.wait()
        for j in range(2, NB):
            x_copy(j, j - 2).start()
        for cp in ffn_copies:
            cp.start()
        wt_ref[0:D, :] = wkv_ref[:, D:2 * D].T
        tiles += k_tiles(xn, K1, G)
        kbar = jnp.concatenate([jnp.sum(t, axis=0, keepdims=True) for t in tiles], axis=1)
        tiles += v_tiles(0, xn, 0, V1)
        n2 = ready(G + V1)
        assert n2 > (G - 1) * nsb
        key_limbs(0, tiles, range(n1, n2), kscs)
        kdiag = jnp.where(own, kbar * (bal_ref[0:1, :] * (sc / TB)), 0.0).astype(bf16)

        wq_copy.wait()
        x_copy(1, 3).wait()
        wt_ref[D:2 * D, :] = (wq_ref[...].astype(f32) * bal_ref[1:2, :]).astype(bf16).T
        tiles += v_tiles(0, xn, V1, G)
        key_limbs(0, tiles, range(n2, npieces), kscs)
        wt_ref[2 * D:2 * D + H, :] = jnp.dot(
            kdiag, wt_ref[D:2 * D, :], preferred_element_type=f32).astype(bf16)
        tiles += q_proj(0, xn)
        norm_paced(1, [_pick(tiles, p) for p in LN_FIRST])
        wo_copy.wait()

        def blk_body(tb, carry):
            @pl.when(tb + 1 < NB)
            def _():
                x_copy(tb + 1, tb - 1).wait()

            for g in range(2):
                rows = pl.ds(pl.multiple_of((tb - 1 + g) * 128, 128), 128)
                wot_ref[tb - 1 + g] = wo_ref[rows, :].T
            xn = xn_ref[...]
            q_proj(tb, xn)
            tiles = k_tiles(xn, 0, G) + v_tiles(tb, xn, 0, G)
            key_limbs(tb, tiles, range(npieces), {})
            norm_paced(jnp.minimum(tb + 1, NB - 1), [_pick(tiles, p) for p in LN_LOOP])
            return carry

        lax.fori_loop(1, NB, blk_body, 0)

    qcols = pl.ds(pl.multiple_of(step * TQ, TQ), TQ)

    def magic(h, blk):
        pk = jnp.concatenate([pk_ref[blk, pl.ds(h, 1), :]] * (TQ // 128), axis=1)
        c = pq_ref[pl.ds(h, 1), qcols] * pk
        return jnp.minimum(jnp.maximum(c, 1.5 * TINY), 1.5 * HUGE)

    def hrows(h):
        return pl.ds(pl.multiple_of(h * DH, DH), DH)

    def fast_body(it, bad):
        ps = {}
        acc = [None] * UNROLL
        lsum = [None] * UNROLL
        first = []

        def wo_part(lo, hi):
            ap_ref[it, lo:hi, :] = jnp.dot(wot_ref[2 * it, lo:hi, :], jnp.concatenate(first, axis=0),
                                           preferred_element_type=f32)

        def qk(u, st):
            h = UNROLL * it + u
            lhs = jnp.concatenate(
                [kl_ref[h, (st + r) * 128 + q * 32:(st + r) * 128 + (q + 1) * 32, :]
                 for r in range(GRP) for q in ORD[r]], axis=0)
            s = jnp.dot(lhs, ql_ref[h, :, qcols], preferred_element_type=i32)
            if st * 128 % TB == 0:
                c = magic(h, st * 128 // TB)
                ps["ab"] = (_bits(c), c + off_ref[pl.ds(h, 1), qcols])
            a, b = ps["ab"]
            for r in range(GRP):
                p = jnp.exp2(_flt(s[r * 128:(r + 1) * 128] + a) - b)
                lc = jnp.sum(p.reshape(16, 8, TQ), axis=0)
                lsum[u] = lc if lsum[u] is None else lsum[u] + lc
                p = jnp.concatenate([p[ORD[r].index(q) * 32:(ORD[r].index(q) + 1) * 32]
                                     for q in range(4)], axis=0)
                ps[(u, st + r)] = p.astype(bf16)

        def pv(u, st):
            h = UNROLL * it + u
            for c in range(st, st + GRP):
                o = jnp.dot(vt_ref[hrows(h), c * 128:(c + 1) * 128], ps.pop((u, c)),
                            preferred_element_type=f32)
                acc[u] = o if acc[u] is None else o + acc[u]
            if st + GRP == NS:
                l = jnp.sum(lsum[u], axis=0, keepdims=True)
                r0 = pl.reciprocal(l, approx=True)
                o = acc[u] * (r0 * (2.0 - l * r0))
                big = jnp.maximum(jnp.maximum(l, r0 * 2.0 ** 40), jnp.abs(o[0:8] + o[8:16]))
                chk_ref[...] = big if u == 0 else jnp.maximum(chk_ref[...], big)
                if u < 8:
                    first.append(o.astype(bf16))
                else:
                    ot_ref[hrows(8 * it + u - 8), :] = o.astype(bf16)

        items = [(u, st) for u in range(UNROLL) for st in range(0, NS, GRP)]
        for t, item in enumerate(items):
            qk(*item)
            if t > 0:
                pv(*items[t - 1])
        wo_part(0, WSPLIT)
        pv(*items[-1])
        wo_part(WSPLIT, D)
        return jnp.maximum(bad, jnp.max(jnp.where(chk_ref[...] <= LIMIT, 0.0, 1.0)))

    bad = lax.fori_loop(0, H // UNROLL, fast_body, jnp.float32(0.0))

    @pl.when(bad > 0.0)
    def _():
        def safe_body(h, carry):
            def scores(blk):
                c = magic(h, blk)
                s = jnp.dot(kl_ref[h, at(blk, 0, TB), :], ql_ref[h, :, qcols],
                            preferred_element_type=i32)
                return _flt(s + _bits(c)) - c

            def max_body(blk, m):
                return jnp.maximum(m, jnp.max(scores(blk), axis=0, keepdims=True))

            m = lax.fori_loop(0, NB, max_body, jnp.full((1, TQ), -jnp.inf, f32))

            def acc_body(blk, la):
                p = jnp.exp2(scores(blk) - m)
                o = jnp.dot(vt_ref[hrows(h), at(blk, 0, TB)], p.astype(bf16),
                            preferred_element_type=f32)
                return la[0] + jnp.sum(p, axis=0, keepdims=True), la[1] + o

            l, acc = lax.fori_loop(0, NB, acc_body,
                                   (jnp.zeros((1, TQ), f32), jnp.zeros((DH, TQ), f32)))
            of_ref[hrows(h), :] = (acc * (1.0 / l)).astype(bf16)
            return carry

        lax.fori_loop(0, H, safe_body, 0)
        for it in range(2):
            ap_ref[it] = jnp.dot(wot_ref[2 * it], of_ref[256 * it:256 * it + 128, :],
                                 preferred_element_type=f32)
            ot_ref[128 * it:128 * (it + 1), :] = of_ref[256 * it + 128:256 * (it + 1), :]

    @pl.when(step == 0)
    def _():
        for cp in ffn_copies:
            cp.wait()

    NJ = TQ // TT
    wdt = wd_ref[...].T
    wodd = jnp.concatenate([wot_ref[1], wot_ref[3]], axis=1)
    ht, hnt, acts = [], [], []

    def trows(j):
        return pl.ds(pl.multiple_of(step * TQ + j * TT, TT), TT)

    for j in range(NJ):
        cs = slice(j * TT, (j + 1) * TT)
        attn = jnp.dot(wodd, ot_ref[:, cs], preferred_element_type=f32)
        attn = attn + (ap_ref[0, :, cs] + ap_ref[1, :, cs])
        ht.append(x_ref[trows(j), :].T.astype(f32) + attn)
        hnt.append(_normalize(ht[j], 0).astype(bf16))

    def down(j):
        if j == NJ - 1:
            y = lax.dot_general(acts[j], wd_ref[...], TN, preferred_element_type=f32)
            o_ref[trows(j), :] = (ht[j].T + y).astype(o_ref.dtype)
        else:
            y = jnp.dot(wdt, acts[j], preferred_element_type=f32)
            o_ref[trows(j), :] = (ht[j] + y).astype(o_ref.dtype).T
        pltpu.make_async_copy(o_ref.at[trows(j), :], o_hbm.at[trows(j), :], sem.at[3]).start()

    for j in range(NJ):
        gate = jnp.dot(wg_ref[...], hnt[j], preferred_element_type=f32)
        up = jnp.dot(wu_ref[...], hnt[j], preferred_element_type=f32)
        acts.append((jax.nn.gelu(gate, approximate=True) * up).astype(bf16))
        if j > 0:
            down(j - 1)
    down(NJ - 1)

    @pl.when(step == pl.num_programs(0) - 1)
    def _():
        pltpu.make_async_copy(o_ref, o_hbm, sem.at[3]).wait()


@jax.jit
def pallas_sequential_preLN__softmax_full_mha__geglu_ffn__prompt_kernel(
    A_x: jax.Array,
    A_wqkv: jax.Array,
    A_wo: jax.Array,
    B_x: jax.Array,
    B_w_gate: jax.Array,
    B_w_up: jax.Array,
    B_w_down: jax.Array,
):
    del B_x
    B, S, D = A_x.shape
    F = B_w_gate.shape[1]
    assert B == 1 and D == H * DH == 512 and S == 4 * TB and H == 2 * UNROLL

    out = pl.pallas_call(
        functools.partial(_kernel, S=S, D=D),
        grid=(S // TQ,),
        in_specs=[pl.BlockSpec(memory_space=pl.ANY)] * 6,
        out_specs=pl.BlockSpec(memory_space=pl.ANY),
        out_shape=jax.ShapeDtypeStruct((S, D), A_x.dtype),
        scratch_shapes=[
            pltpu.VMEM((S, D), bf16),
            pltpu.VMEM((D, 2 * D), bf16),
            pltpu.VMEM((D, D), bf16),
            pltpu.VMEM((D, D), bf16),
            pltpu.VMEM((F, D), bf16),
            pltpu.VMEM((F, D), bf16),
            pltpu.VMEM((F, D), bf16),
            pltpu.SemaphoreType.DMA((5,)),
            pltpu.VMEM((2 * D + H, D), bf16),
            pltpu.VMEM((D // 128, D, 128), bf16),
            pltpu.VMEM((TB, D), bf16),
            pltpu.VMEM((H, S, 128), i8),
            pltpu.VMEM((H, 128, S), i8),
            pltpu.VMEM((D, S), bf16),
            pltpu.VMEM((H, S), f32),
            pltpu.VMEM((H, S), f32),
            pltpu.VMEM((S // TB, H, 128), f32),
            pltpu.VMEM((2, D), f32),
            pltpu.VMEM((D // 2, TQ), bf16),
            pltpu.VMEM((2, D, TQ), f32),
            pltpu.VMEM((D, TQ), bf16),
            pltpu.VMEM((8, TQ), f32),
            pltpu.VMEM((S, D), A_x.dtype),
        ],
        compiler_params=pltpu.CompilerParams(
            dimension_semantics=("arbitrary",),
            vmem_limit_bytes=100 * 1024 * 1024,
        ),
    )(A_x.reshape(S, D), A_wqkv, A_wo, B_w_gate.T, B_w_up.T, B_w_down)
    return out.reshape(B, S, D)
```

```python
import functools
import math

import jax
import jax.numpy as jnp
from jax import lax
import jax.experimental.pallas as pl
import jax.experimental.pallas.tpu as pltpu

f32 = jnp.float32
bf16 = jnp.bfloat16
i32 = jnp.int32
i8 = jnp.int8

H = 32
DH = 16
TQ = 512
TB = 512
UNROLL = 16
GRP = 2
ORD = ((1, 3, 2, 0), (2, 0, 1, 3))
WSPLIT = 144
TT = 128
KSUB = 32
K1 = 3
V1 = 2
TSPAN = 6.0
EARLY = 0.3
LN_FIRST = tuple(6.1 + i * 0.15 for i in range(32))
LN_LOOP = tuple(0.05 + i * 0.225 for i in range(32))

EPS = 1e-5
LOG2E = 1.4426950408889634
RND = 12582912.0
C2 = 28.0
MAX_BAL = 2.0 ** 12
SHIFT = 32.0
LIMIT = 2.0 ** 100
TINY = 2.0 ** -120
HUGE = 2.0 ** 120
EXP_MASK = 0x7F800000
NT = (((1,), (1,)), ((), ()))
TN = (((0,), (0,)), ((), ()))


def _bits(x):
    return lax.bitcast_convert_type(x, i32)


def _flt(x):
    return lax.bitcast_convert_type(x, f32)


def _normalize(x, axis):
    mu = jnp.mean(x, axis=axis, keepdims=True)
    xc = x - mu
    var = jnp.mean(xc * xc, axis=axis, keepdims=True)
    return xc * lax.rsqrt(var + EPS)


def _pow2_floor_bits(z):
    return _bits(jnp.minimum(jnp.maximum(z, TINY), HUGE)) & EXP_MASK


def _half_inv(pbits):
    return _flt((253 << 23) - pbits)


def _after(x, tie):
    return jnp.minimum(x, jnp.maximum(x, tie))


def _split(arr):
    return [arr[:, j * 128:(j + 1) * 128] for j in range(arr.shape[1] // 128)]


def _pick(tiles, pos):
    tile = int(pos)
    row = int((pos - tile) * TB) // 8 * 8
    return tiles[tile][row:row + 1, :]


def _kernel(x_hbm, wqkv_hbm, wo_hbm, wg_hbm, wu_hbm, wd_hbm, o_hbm,
            x_ref, wkv_ref, wq_ref, wo_ref, wg_ref, wu_ref, wd_ref, sem,
            wt_ref, wot_ref, xn_ref, kl_ref, ql_ref, vt_ref, pq_ref, off_ref, pk_ref, bal_ref,
            ot_ref, ap_ref, of_ref, chk_ref, o_ref, *, S, D):
    step = pl.program_id(0)
    NB = S // TB
    NS = S // 128
    G = D // 128

    def at(tb, off, size):
        start = tb * TB + off
        if isinstance(start, int):
            return slice(start, start + size)
        return pl.ds(pl.multiple_of(start, math.gcd(TB, off)), size)

    def x_copy(tb, s):
        return pltpu.make_async_copy(x_hbm.at[at(tb, 0, TB), :], x_ref.at[at(tb, 0, TB), :],
                                     sem.at[s])

    ca = K1 * 128
    wk_copy = pltpu.make_async_copy(wqkv_hbm.at[:, D:D + ca], wkv_ref.at[:, 0:ca], sem.at[1])
    wv_copy = pltpu.make_async_copy(wqkv_hbm.at[:, D + ca:3 * D], wkv_ref.at[:, ca:2 * D], sem.at[2])
    wq_copy = pltpu.make_async_copy(wqkv_hbm.at[:, 0:D], wq_ref, sem.at[3])
    wo_copy = pltpu.make_async_copy(wo_hbm, wo_ref, sem.at[4])
    ffn_copies = [pltpu.make_async_copy(src, dst, sem.at[2])
                  for src, dst in ((wg_hbm, wg_ref), (wu_hbm, wu_ref), (wd_hbm, wd_ref))]

    @pl.when(step == 0)
    def _():
        x_copy(0, 0).start()
        wk_copy.start()
        wv_copy.start()
        wq_copy.start()
        x_copy(1, 3).start()
        wo_copy.start()
        x_copy(0, 0).wait()

        own8 = (lax.broadcasted_iota(i32, (8, 128), 1) // DH) == lax.broadcasted_iota(i32, (8, 128), 0)
        own = (lax.broadcasted_iota(i32, (H, D), 1) // DH) == lax.broadcasted_iota(i32, (H, D), 0)
        lane = lax.broadcasted_iota(i32, (KSUB // 4, 128), 1)
        sc = DH ** -0.5 * LOG2E
        cq = sc / 7.0
        nsb = TB // KSUB
        npieces = G * nsb

        def key_limbs(tb, tiles, pieces, kscs):
            for idx in pieces:
                g, sb = idx // nsb, idx % nsb
                if g not in kscs:
                    gl = slice(g * 128, (g + 1) * 128)
                    kabs = jnp.max(jnp.abs(tiles[g]), axis=0, keepdims=True)
                    bal = bal_ref[0:1, gl]
                    kmax = jnp.max(jnp.where(own8, kabs * bal, 0.0), axis=1, keepdims=True)
                    pk = _pow2_floor_bits(kmax * (1.0 / 127.25))
                    pk_ref[tb, g * 8:(g + 1) * 8, :] = jnp.broadcast_to(
                        _flt(pk) * (1.5 * 2.0 ** 25), (8, 128))
                    kscs[g] = bal * jnp.max(jnp.where(own8, _half_inv(pk), 0.0), axis=0, keepdims=True)
                ksc = _after(kscs[g], _pick(tiles, 1.0 + idx * TSPAN / npieces))
                ks = tiles[g][sb * KSUB:(sb + 1) * KSUB] * ksc
                fh = jnp.floor(ks + 0.5)
                yh = fh + RND
                yl = (ks - fh) * C2 + RND
                kh = pltpu.bitcast(_bits(yh).astype(i8), i32)
                kl = pltpu.bitcast(_bits(yl).astype(i8), i32)
                cur = [kl] + [pltpu.roll(kh, DH * j, 1) for j in range(1, 8)]
                for bit in (1, 2, 4):
                    on = (lane & (DH * bit)) != 0
                    cur = [jnp.where(on, cur[(j + bit) % 8], cur[j]) for j in range(8)]
                for j in range(8):
                    kl_ref[g * 8 + (-j) % 8, at(tb, sb * KSUB, KSUB), :] = pltpu.bitcast(cur[j], i8)

        def balance(lo, hi):
            for g in range(lo, hi):
                gl = slice(g * 128, (g + 1) * 128)
                wabs = jnp.sum(jnp.abs(wkv_ref[:, gl].astype(f32)), axis=0, keepdims=True)
                top = jnp.max(jnp.where(own8, wabs, 0.0), axis=1, keepdims=True)
                top = jnp.max(jnp.where(own8, top, 0.0), axis=0, keepdims=True)
                ratio = jnp.clip(top / jnp.maximum(wabs, TINY), 1.0, MAX_BAL)
                pb = _bits(ratio) & EXP_MASK
                bal_ref[0:1, gl] = _flt(pb)
                bal_ref[1:2, gl] = _flt((254 << 23) - pb)

        def ready(ntiles):
            return len([i for i in range(npieces) if 1.0 + i * TSPAN / npieces < ntiles - EARLY])

        def norm_paced(tb, ties):
            rs = TB // len(ties)
            for i, tie in enumerate(ties):
                one = jnp.concatenate([_after(jnp.ones((1, 128), f32), tie)] * G, axis=1)
                xf = x_ref[at(tb, i * rs, rs), :].astype(f32) * one
                xn_ref[i * rs:(i + 1) * rs, :] = _normalize(xf, -1).astype(bf16)

        def k_tiles(xn, lo, hi):
            return _split(jnp.dot(xn, wkv_ref[:, lo * 128:hi * 128], preferred_element_type=f32))

        def v_tiles(tb, xn, lo, hi):
            vt = lax.dot_general(wt_ref[0:D, :], xn[lo * 128:hi * 128], NT,
                                 preferred_element_type=f32)
            vt_ref[:, at(tb, lo * 128, (hi - lo) * 128)] = vt.astype(bf16)
            return _split(vt)

        def q_proj(tb, xn):
            qt = lax.dot_general(wt_ref[D:2 * D + H, :], xn, NT, preferred_element_type=f32)
            off_ref[:, at(tb, 0, TB)] = qt[D:D + H, :] + SHIFT
            for j in range(TB // 128):
                cols = at(tb, j * 128, 128)
                for h in range(H):
                    qh = qt[h * DH:(h + 1) * DH, j * 128:(j + 1) * 128]
                    qmax = jnp.max(jnp.abs(qh), axis=0, keepdims=True)
                    pq = _pow2_floor_bits(qmax * (cq / 124.0))
                    pq_ref[h:h + 1, cols] = _flt(pq)
                    xq = qh * (_half_inv(pq) * cq)
                    fb = jnp.floor(xq + 0.5)
                    yb = fb + RND
                    yr = (xq - fb) * 7.0 + yb
                    ya = xq * (7.0 / C2) + RND
                    bb = jnp.concatenate([_bits(yb), _bits(yb)], axis=0).astype(i8)
                    pair = [_bits(ya), _bits(yr)] if h % 2 == 0 else [_bits(yr), _bits(ya)]
                    ar = jnp.concatenate(pair, axis=0).astype(i8)
                    for ps in range(4):
                        ql_ref[h, ps * 32:(ps + 1) * 32, cols] = ar if ps == (h % 8) // 2 else bb
            return _split(qt)

        xn = _normalize(x_ref[0:TB, :].astype(f32), -1).astype(bf16)
        wk_copy.wait()
        balance(0, K1)
        kscs = {}
        tiles = k_tiles(xn, 0, K1)
        n1 = ready(K1)
        key_limbs(0, tiles, range(n1), kscs)

        wv_copy.wait()
        for j in range(2, NB):
            x_copy(j, j - 2).start()
        for cp in ffn_copies:
            cp.start()
        balance(K1, G)
        wt_ref[0:D, :] = wkv_ref[:, D:2 * D].T
        tiles += k_tiles(xn, K1, G)
        kbar = jnp.concatenate([jnp.sum(t, axis=0, keepdims=True) for t in tiles], axis=1)
        tiles += v_tiles(0, xn, 0, V1)
        n2 = ready(G + V1)
        key_limbs(0, tiles, range(n1, n2), kscs)
        kdiag = jnp.where(own, kbar * (bal_ref[0:1, :] * (sc / TB)), 0.0).astype(bf16)

        wq_copy.wait()
        x_copy(1, 3).wait()
        wt_ref[D:2 * D, :] = (wq_ref[...].astype(f32) * bal_ref[1:2, :]).astype(bf16).T
        tiles += v_tiles(0, xn, V1, G)
        key_limbs(0, tiles, range(n2, npieces), kscs)
        wt_ref[2 * D:2 * D + H, :] = jnp.dot(
            kdiag, wt_ref[D:2 * D, :], preferred_element_type=f32).astype(bf16)
        tiles += q_proj(0, xn)
        norm_paced(1, [_pick(tiles, p) for p in LN_FIRST])
        wo_copy.wait()

        def blk_body(tb, carry):
            @pl.when(tb + 1 < NB)
            def _():
                x_copy(tb + 1, tb - 1).wait()

            for g in range(2):
                rows = pl.ds(pl.multiple_of((tb - 1 + g) * 128, 128), 128)
                wot_ref[tb - 1 + g] = wo_ref[rows, :].T
            xn = xn_ref[...]
            q_proj(tb, xn)
            tiles = k_tiles(xn, 0, G) + v_tiles(tb, xn, 0, G)
            key_limbs(tb, tiles, range(npieces), {})
            norm_paced(jnp.minimum(tb + 1, NB - 1), [_pick(tiles, p) for p in LN_LOOP])
            return carry

        lax.fori_loop(1, NB, blk_body, 0)

    qcols = pl.ds(pl.multiple_of(step * TQ, TQ), TQ)

    def magic(h, blk):
        pk = jnp.concatenate([pk_ref[blk, pl.ds(h, 1), :]] * (TQ // 128), axis=1)
        c = pq_ref[pl.ds(h, 1), qcols] * pk
        return jnp.minimum(jnp.maximum(c, 1.5 * TINY), 1.5 * HUGE)

    def hrows(h):
        return pl.ds(pl.multiple_of(h * DH, DH), DH)

    def fast_body(it, bad):
        ps = {}
        acc = [None] * UNROLL
        lsum = [None] * UNROLL
        first = []

        def wo_part(lo, hi):
            ap_ref[it, lo:hi, :] = jnp.dot(wot_ref[2 * it, lo:hi, :], jnp.concatenate(first, axis=0),
                                           preferred_element_type=f32)

        def qk(u, st):
            h = UNROLL * it + u
            lhs = jnp.concatenate(
                [kl_ref[h, (st + r) * 128 + q * 32:(st + r) * 128 + (q + 1) * 32, :]
                 for r in range(GRP) for q in ORD[r]], axis=0)
            s = jnp.dot(lhs, ql_ref[h, :, qcols], preferred_element_type=i32)
            if st * 128 % TB == 0:
                c = magic(h, st * 128 // TB)
                ps["ab"] = (_bits(c), c + off_ref[pl.ds(h, 1), qcols])
            a, b = ps["ab"]
            for r in range(GRP):
                p = jnp.exp2(_flt(s[r * 128:(r + 1) * 128] + a) - b)
                lc = jnp.sum(p.reshape(16, 8, TQ), axis=0)
                lsum[u] = lc if lsum[u] is None else lsum[u] + lc
                p = jnp.concatenate([p[ORD[r].index(q) * 32:(ORD[r].index(q) + 1) * 32]
                                     for q in range(4)], axis=0)
                ps[(u, st + r)] = p.astype(bf16)

        def pv(u, st):
            h = UNROLL * it + u
            for c in range(st, st + GRP):
                o = jnp.dot(vt_ref[hrows(h), c * 128:(c + 1) * 128], ps.pop((u, c)),
                            preferred_element_type=f32)
                acc[u] = o if acc[u] is None else o + acc[u]
            if st + GRP == NS:
                l = jnp.sum(lsum[u], axis=0, keepdims=True)
                r0 = pl.reciprocal(l, approx=True)
                o = acc[u] * (r0 * (2.0 - l * r0))
                big = jnp.maximum(jnp.maximum(l, r0 * 2.0 ** 40), jnp.abs(o[0:8] + o[8:16]))
                chk_ref[...] = big if u == 0 else jnp.maximum(chk_ref[...], big)
                if u < 8:
                    first.append(o.astype(bf16))
                else:
                    ot_ref[hrows(8 * it + u - 8), :] = o.astype(bf16)

        items = [(u, st) for u in range(UNROLL) for st in range(0, NS, GRP)]
        for t, item in enumerate(items):
            qk(*item)
            if t > 0:
                pv(*items[t - 1])
        wo_part(0, WSPLIT)
        pv(*items[-1])
        wo_part(WSPLIT, D)
        return jnp.maximum(bad, jnp.max(jnp.where(chk_ref[...] <= LIMIT, 0.0, 1.0)))

    bad = lax.fori_loop(0, H // UNROLL, fast_body, jnp.float32(0.0))

    @pl.when(bad > 0.0)
    def _():
        def safe_body(h, carry):
            def scores(blk):
                c = magic(h, blk)
                s = jnp.dot(kl_ref[h, at(blk, 0, TB), :], ql_ref[h, :, qcols],
                            preferred_element_type=i32)
                return _flt(s + _bits(c)) - c

            def max_body(blk, m):
                return jnp.maximum(m, jnp.max(scores(blk), axis=0, keepdims=True))

            m = lax.fori_loop(0, NB, max_body, jnp.full((1, TQ), -jnp.inf, f32))

            def acc_body(blk, la):
                p = jnp.exp2(scores(blk) - m)
                o = jnp.dot(vt_ref[hrows(h), at(blk, 0, TB)], p.astype(bf16),
                            preferred_element_type=f32)
                return la[0] + jnp.sum(p, axis=0, keepdims=True), la[1] + o

            l, acc = lax.fori_loop(0, NB, acc_body,
                                   (jnp.zeros((1, TQ), f32), jnp.zeros((DH, TQ), f32)))
            of_ref[hrows(h), :] = (acc * (1.0 / l)).astype(bf16)
            return carry

        lax.fori_loop(0, H, safe_body, 0)
        for it in range(2):
            ap_ref[it] = jnp.dot(wot_ref[2 * it], of_ref[256 * it:256 * it + 128, :],
                                 preferred_element_type=f32)
            ot_ref[128 * it:128 * (it + 1), :] = of_ref[256 * it + 128:256 * (it + 1), :]

    @pl.when(step == 0)
    def _():
        for cp in ffn_copies:
            cp.wait()

    NJ = TQ // TT
    wdt = wd_ref[...].T
    wodd = jnp.concatenate([wot_ref[1], wot_ref[3]], axis=1)
    ht, hnt, acts = [], [], []

    def trows(j):
        return pl.ds(pl.multiple_of(step * TQ + j * TT, TT), TT)

    for j in range(NJ):
        cs = slice(j * TT, (j + 1) * TT)
        attn = jnp.dot(wodd, ot_ref[:, cs], preferred_element_type=f32)
        attn = attn + (ap_ref[0, :, cs] + ap_ref[1, :, cs])
        ht.append(x_ref[trows(j), :].T.astype(f32) + attn)
        hnt.append(_normalize(ht[j], 0).astype(bf16))

    def down(j):
        if j == NJ - 1:
            y = lax.dot_general(acts[j], wd_ref[...], TN, preferred_element_type=f32)
            o_ref[trows(j), :] = (ht[j].T + y).astype(o_ref.dtype)
        else:
            y = jnp.dot(wdt, acts[j], preferred_element_type=f32)
            o_ref[trows(j), :] = (ht[j] + y).astype(o_ref.dtype).T
        pltpu.make_async_copy(o_ref.at[trows(j), :], o_hbm.at[trows(j), :], sem.at[3]).start()

    for j in range(NJ):
        gate = jnp.dot(wg_ref[...], hnt[j], preferred_element_type=f32)
        up = jnp.dot(wu_ref[...], hnt[j], preferred_element_type=f32)
        acts.append((jax.nn.gelu(gate, approximate=True) * up).astype(bf16))
        if j > 0:
            down(j - 1)
    down(NJ - 1)

    @pl.when(step == pl.num_programs(0) - 1)
    def _():
        pltpu.make_async_copy(o_ref, o_hbm, sem.at[3]).wait()


@jax.jit
def pallas_sequential_preLN__softmax_full_mha__geglu_ffn__prompt_kernel(
    A_x: jax.Array,
    A_wqkv: jax.Array,
    A_wo: jax.Array,
    B_x: jax.Array,
    B_w_gate: jax.Array,
    B_w_up: jax.Array,
    B_w_down: jax.Array,
):
    del B_x
    B, S, D = A_x.shape
    F = B_w_gate.shape[1]
    assert B == 1 and D == H * DH == 512 and S == 4 * TB and H == 2 * UNROLL

    out = pl.pallas_call(
        functools.partial(_kernel, S=S, D=D),
        grid=(S // TQ,),
        in_specs=[pl.BlockSpec(memory_space=pl.ANY)] * 6,
        out_specs=pl.BlockSpec(memory_space=pl.ANY),
        out_shape=jax.ShapeDtypeStruct((S, D), A_x.dtype),
        scratch_shapes=[
            pltpu.VMEM((S, D), bf16),
            pltpu.VMEM((D, 2 * D), bf16),
            pltpu.VMEM((D, D), bf16),
            pltpu.VMEM((D, D), bf16),
            pltpu.VMEM((F, D), bf16),
            pltpu.VMEM((F, D), bf16),
            pltpu.VMEM((F, D), bf16),
            pltpu.SemaphoreType.DMA((5,)),
            pltpu.VMEM((2 * D + H, D), bf16),
            pltpu.VMEM((D // 128, D, 128), bf16),
            pltpu.VMEM((TB, D), bf16),
            pltpu.VMEM((H, S, 128), i8),
            pltpu.VMEM((H, 128, S), i8),
            pltpu.VMEM((D, S), bf16),
            pltpu.VMEM((H, S), f32),
            pltpu.VMEM((H, S), f32),
            pltpu.VMEM((S // TB, H, 128), f32),
            pltpu.VMEM((2, D), f32),
            pltpu.VMEM((D // 2, TQ), bf16),
            pltpu.VMEM((2, D, TQ), f32),
            pltpu.VMEM((D, TQ), bf16),
            pltpu.VMEM((8, TQ), f32),
            pltpu.VMEM((S, D), A_x.dtype),
        ],
        compiler_params=pltpu.CompilerParams(
            dimension_semantics=("arbitrary",),
            vmem_limit_bytes=100 * 1024 * 1024,
        ),
    )(A_x.reshape(S, D), A_wqkv, A_wo, B_w_gate.T, B_w_up.T, B_w_down)
    return out.reshape(B, S, D)
```

```python
import functools
import math

import jax
import jax.numpy as jnp
from jax import lax
import jax.experimental.pallas as pl
import jax.experimental.pallas.tpu as pltpu

f32 = jnp.float32
bf16 = jnp.bfloat16
i32 = jnp.int32
i8 = jnp.int8

H = 32
DH = 16
TQ = 512
TB = 512
UNROLL = 16
GRP = 2
ORD = ((1, 3, 2, 0), (2, 0, 1, 3))
WSPLIT = 144
TT = 128
KSUB = 32
K1 = 3
V1 = 2
TSPAN = 6.0
EARLY = 0.3
LN_FIRST = tuple(6.1 + i * 0.15 for i in range(32))
LN_LOOP = tuple(0.05 + i * 0.225 for i in range(32))

EPS = 1e-5
LOG2E = 1.4426950408889634
RND = 12582912.0
C2 = 28.0
MAX_BAL = 2.0 ** 12
SHIFT = 32.0
LIMIT = 2.0 ** 100
C_MAX = 1.5 * 2.0 ** 12
TINY = 2.0 ** -100
HUGE = 2.0 ** 100
EXP_MASK = 0x7F800000
NT = (((1,), (1,)), ((), ()))
TN = (((0,), (0,)), ((), ()))


def _bits(x):
    return lax.bitcast_convert_type(x, i32)


def _flt(x):
    return lax.bitcast_convert_type(x, f32)


def _normalize(x, axis):
    mu = jnp.mean(x, axis=axis, keepdims=True)
    xc = x - mu
    var = jnp.mean(xc * xc, axis=axis, keepdims=True)
    return xc * lax.rsqrt(var + EPS)


def _pow2_floor_bits(z):
    return _bits(jnp.minimum(jnp.maximum(z, TINY), HUGE)) & EXP_MASK


def _half_inv(pbits):
    return _flt((253 << 23) - pbits)


def _after(x, tie):
    return jnp.minimum(x, jnp.maximum(x, tie))


def _split(arr):
    return [arr[:, j * 128:(j + 1) * 128] for j in range(arr.shape[1] // 128)]


def _pick(tiles, pos):
    tile = int(pos)
    row = int((pos - tile) * TB) // 8 * 8
    return tiles[tile][row:row + 1, :]


def _kernel(x_hbm, wqkv_hbm, wo_hbm, wg_hbm, wu_hbm, wd_hbm, o_hbm,
            x_ref, wkv_ref, wq_ref, wo_ref, wg_ref, wu_ref, wd_ref, sem,
            wt_ref, wot_ref, xn_ref, kl_ref, ql_ref, vt_ref, pq_ref, off_ref, pk_ref, bal_ref,
            ot_ref, ap_ref, of_ref, kb_ref, qb_ref, chk_ref, o_ref, *, S, D):
    step = pl.program_id(0)
    NB = S // TB
    NS = S // 128
    G = D // 128

    def at(tb, off, size):
        start = tb * TB + off
        if isinstance(start, int):
            return slice(start, start + size)
        return pl.ds(pl.multiple_of(start, math.gcd(TB, off)), size)

    def x_copy(tb, s):
        return pltpu.make_async_copy(x_hbm.at[at(tb, 0, TB), :], x_ref.at[at(tb, 0, TB), :],
                                     sem.at[s])

    ca = K1 * 128
    wk_copy = pltpu.make_async_copy(wqkv_hbm.at[:, D:D + ca], wkv_ref.at[:, 0:ca], sem.at[1])
    wv_copy = pltpu.make_async_copy(wqkv_hbm.at[:, D + ca:3 * D], wkv_ref.at[:, ca:2 * D], sem.at[2])
    wq_copy = pltpu.make_async_copy(wqkv_hbm.at[:, 0:D], wq_ref, sem.at[3])
    wo_copy = pltpu.make_async_copy(wo_hbm, wo_ref, sem.at[4])
    ffn_copies = [pltpu.make_async_copy(src, dst, sem.at[2])
                  for src, dst in ((wg_hbm, wg_ref), (wu_hbm, wu_ref), (wd_hbm, wd_ref))]

    @pl.when(step == 0)
    def _():
        x_copy(0, 0).start()
        wk_copy.start()
        wv_copy.start()
        wq_copy.start()
        x_copy(1, 3).start()
        wo_copy.start()
        x_copy(0, 0).wait()

        own8 = (lax.broadcasted_iota(i32, (8, 128), 1) // DH) == lax.broadcasted_iota(i32, (8, 128), 0)
        own = (lax.broadcasted_iota(i32, (H, D), 1) // DH) == lax.broadcasted_iota(i32, (H, D), 0)
        lane = lax.broadcasted_iota(i32, (KSUB // 4, 128), 1)
        sc = DH ** -0.5 * LOG2E
        cq = sc / 7.0
        nsb = TB // KSUB
        npieces = G * nsb

        def key_limbs(tb, tiles, pieces, kscs):
            for idx in pieces:
                g, sb = idx // nsb, idx % nsb
                if g not in kscs:
                    gl = slice(g * 128, (g + 1) * 128)
                    kabs = jnp.max(jnp.abs(tiles[g]), axis=0, keepdims=True)
                    bal = bal_ref[0:1, gl]
                    kmax = jnp.max(jnp.where(own8, kabs * bal, 0.0), axis=1, keepdims=True)
                    pk = _pow2_floor_bits(kmax * (1.0 / 127.25))
                    pk_ref[tb, g * 8:(g + 1) * 8, :] = jnp.broadcast_to(
                        _flt(pk) * (1.5 * 2.0 ** 25), (8, 128))
                    kscs[g] = bal * jnp.max(jnp.where(own8, _half_inv(pk), 0.0), axis=0, keepdims=True)
                ksc = _after(kscs[g], _pick(tiles, 1.0 + idx * TSPAN / npieces))
                ks = tiles[g][sb * KSUB:(sb + 1) * KSUB] * ksc
                fh = jnp.floor(ks + 0.5)
                yh = fh + RND
                yl = (ks - fh) * C2 + RND
                kh = pltpu.bitcast(_bits(yh).astype(i8), i32)
                kl = pltpu.bitcast(_bits(yl).astype(i8), i32)
                cur = [kl] + [pltpu.roll(kh, DH * j, 1) for j in range(1, 8)]
                for bit in (1, 2, 4):
                    on = (lane & (DH * bit)) != 0
                    cur = [jnp.where(on, cur[(j + bit) % 8], cur[j]) for j in range(8)]
                for j in range(8):
                    kl_ref[g * 8 + (-j) % 8, at(tb, sb * KSUB, KSUB), :] = pltpu.bitcast(cur[j], i8)

        def balance(lo, hi):
            for g in range(lo, hi):
                gl = slice(g * 128, (g + 1) * 128)
                wabs = jnp.sum(jnp.abs(wkv_ref[:, gl].astype(f32)), axis=0, keepdims=True)
                top = jnp.max(jnp.where(own8, wabs, 0.0), axis=1, keepdims=True)
                top = jnp.max(jnp.where(own8, top, 0.0), axis=0, keepdims=True)
                ratio = jnp.clip(top / jnp.maximum(wabs, TINY), 1.0, MAX_BAL)
                pb = _bits(ratio) & EXP_MASK
                bal_ref[0:1, gl] = _flt(pb)
                bal_ref[1:2, gl] = _flt((254 << 23) - pb)

        def ready(ntiles):
            return len([i for i in range(npieces) if 1.0 + i * TSPAN / npieces < ntiles - EARLY])

        def norm_paced(tb, ties):
            rs = TB // len(ties)
            for i, tie in enumerate(ties):
                one = jnp.concatenate([_after(jnp.ones((1, 128), f32), tie)] * G, axis=1)
                xf = x_ref[at(tb, i * rs, rs), :].astype(f32) * one
                xn_ref[i * rs:(i + 1) * rs, :] = _normalize(xf, -1).astype(bf16)

        def k_tiles(xn, lo, hi):
            return _split(jnp.dot(xn, wkv_ref[:, lo * 128:hi * 128], preferred_element_type=f32))

        def v_tiles(tb, xn, lo, hi):
            vt = lax.dot_general(wt_ref[0:D, :], xn[lo * 128:hi * 128], NT,
                                 preferred_element_type=f32)
            vt_ref[:, at(tb, lo * 128, (hi - lo) * 128)] = vt.astype(bf16)
            return _split(vt)

        def q_proj(tb, xn):
            qt = lax.dot_general(wt_ref[D:2 * D + H, :], xn, NT, preferred_element_type=f32)
            off_ref[:, at(tb, 0, TB)] = qt[D:D + H, :] + SHIFT
            for j in range(TB // 128):
                cols = at(tb, j * 128, 128)
                for h in range(H):
                    qh = qt[h * DH:(h + 1) * DH, j * 128:(j + 1) * 128]
                    qmax = jnp.max(jnp.abs(qh), axis=0, keepdims=True)
                    pq = _pow2_floor_bits(qmax * (cq / 124.0))
                    pq_ref[h:h + 1, cols] = _flt(pq)
                    xq = qh * (_half_inv(pq) * cq)
                    fb = jnp.floor(xq + 0.5)
                    yb = fb + RND
                    yr = (xq - fb) * 7.0 + yb
                    ya = xq * (7.0 / C2) + RND
                    bb = jnp.concatenate([_bits(yb), _bits(yb)], axis=0).astype(i8)
                    pair = [_bits(ya), _bits(yr)] if h % 2 == 0 else [_bits(yr), _bits(ya)]
                    ar = jnp.concatenate(pair, axis=0).astype(i8)
                    for ps in range(4):
                        ql_ref[h, ps * 32:(ps + 1) * 32, cols] = ar if ps == (h % 8) // 2 else bb
            return _split(qt)

        xn = _normalize(x_ref[0:TB, :].astype(f32), -1).astype(bf16)
        wk_copy.wait()
        balance(0, K1)
        kscs = {}
        tiles = k_tiles(xn, 0, K1)
        n1 = ready(K1)
        key_limbs(0, tiles, range(n1), kscs)

        wv_copy.wait()
        for j in range(2, NB):
            x_copy(j, j - 2).start()
        for cp in ffn_copies:
            cp.start()
        balance(K1, G)
        wt_ref[0:D, :] = wkv_ref[:, D:2 * D].T
        tiles += k_tiles(xn, K1, G)
        kbar = jnp.concatenate([jnp.sum(t, axis=0, keepdims=True) for t in tiles], axis=1)
        tiles += v_tiles(0, xn, 0, V1)
        n2 = ready(G + V1)
        key_limbs(0, tiles, range(n1, n2), kscs)
        kdiag = jnp.where(own, kbar * (bal_ref[0:1, :] * (sc / TB)), 0.0).astype(bf16)

        wq_copy.wait()
        x_copy(1, 3).wait()
        wt_ref[D:2 * D, :] = (wq_ref[...].astype(f32) * bal_ref[1:2, :]).astype(bf16).T
        tiles += v_tiles(0, xn, V1, G)
        key_limbs(0, tiles, range(n2, npieces), kscs)
        wt_ref[2 * D:2 * D + H, :] = jnp.dot(
            kdiag, wt_ref[D:2 * D, :], preferred_element_type=f32).astype(bf16)
        tiles += q_proj(0, xn)
        norm_paced(1, [_pick(tiles, p) for p in LN_FIRST])
        wo_copy.wait()

        def blk_body(tb, carry):
            @pl.when(tb + 1 < NB)
            def _():
                x_copy(tb + 1, tb - 1).wait()

            for g in range(2):
                rows = pl.ds(pl.multiple_of((tb - 1 + g) * 128, 128), 128)
                wot_ref[tb - 1 + g] = wo_ref[rows, :].T
            xn = xn_ref[...]
            q_proj(tb, xn)
            tiles = k_tiles(xn, 0, G) + v_tiles(tb, xn, 0, G)
            key_limbs(tb, tiles, range(npieces), {})
            norm_paced(jnp.minimum(tb + 1, NB - 1), [_pick(tiles, p) for p in LN_LOOP])
            return carry

        lax.fori_loop(1, NB, blk_body, 0)

    qcols = pl.ds(pl.multiple_of(step * TQ, TQ), TQ)

    def magic(h, blk):
        pk = jnp.concatenate([pk_ref[blk, pl.ds(h, 1), :]] * (TQ // 128), axis=1)
        c = pq_ref[pl.ds(h, 1), qcols] * pk
        return jnp.minimum(jnp.maximum(c, 1.5 * TINY), 1.5 * HUGE)

    def hrows(h):
        return pl.ds(pl.multiple_of(h * DH, DH), DH)

    def fast_body(it, bad):
        ps = {}
        acc = [None] * UNROLL
        lsum = [None] * UNROLL
        first = []

        def wo_part(lo, hi):
            ap_ref[it, lo:hi, :] = jnp.dot(wot_ref[2 * it, lo:hi, :], jnp.concatenate(first, axis=0),
                                           preferred_element_type=f32)

        def qk(u, st):
            h = UNROLL * it + u
            lhs = jnp.concatenate(
                [kl_ref[h, (st + r) * 128 + q * 32:(st + r) * 128 + (q + 1) * 32, :]
                 for r in range(GRP) for q in ORD[r]], axis=0)
            s = jnp.dot(lhs, ql_ref[h, :, qcols], preferred_element_type=i32)
            if st * 128 % TB == 0:
                c = magic(h, st * 128 // TB)
                ps["ab"] = (_bits(c), c + off_ref[pl.ds(h, 1), qcols])
            a, b = ps["ab"]
            for r in range(GRP):
                p = jnp.exp2(_flt(s[r * 128:(r + 1) * 128] + a) - b)
                lc = jnp.sum(p.reshape(16, 8, TQ), axis=0)
                lsum[u] = lc if lsum[u] is None else lsum[u] + lc
                p = jnp.concatenate([p[ORD[r].index(q) * 32:(ORD[r].index(q) + 1) * 32]
                                     for q in range(4)], axis=0)
                ps[(u, st + r)] = p.astype(bf16)

        def pv(u, st):
            h = UNROLL * it + u
            for c in range(st, st + GRP):
                o = jnp.dot(vt_ref[hrows(h), c * 128:(c + 1) * 128], ps.pop((u, c)),
                            preferred_element_type=f32)
                acc[u] = o if acc[u] is None else o + acc[u]
            if st + GRP == NS:
                l = jnp.sum(lsum[u], axis=0, keepdims=True)
                r0 = pl.reciprocal(l, approx=True)
                o = acc[u] * (r0 * (2.0 - l * r0))
                big = jnp.maximum(jnp.maximum(l, r0 * 2.0 ** 40), jnp.abs(o[0:8] + o[8:16]))
                chk_ref[...] = big if u == 0 else jnp.maximum(chk_ref[...], big)
                if u < 8:
                    first.append(o.astype(bf16))
                else:
                    ot_ref[hrows(8 * it + u - 8), :] = o.astype(bf16)

        items = [(u, st) for u in range(UNROLL) for st in range(0, NS, GRP)]
        for t, item in enumerate(items):
            qk(*item)
            if t > 0:
                pv(*items[t - 1])
        wo_part(0, WSPLIT)
        pv(*items[-1])
        wo_part(WSPLIT, D)
        heads = pl.ds(pl.multiple_of(it * UNROLL, UNROLL), UNROLL)
        pk = functools.reduce(jnp.maximum, [pk_ref[blk, heads, :] for blk in range(NB)])
        pq = functools.reduce(jnp.maximum, _split(pq_ref[heads, qcols]))
        coarse = jnp.where(pq * pk <= C_MAX, 0.0, 1.0)
        unsafe = functools.reduce(jnp.maximum, _split(jnp.where(chk_ref[...] <= LIMIT, 0.0, 1.0)))
        flag = jnp.maximum(jnp.maximum(coarse[0:8], coarse[8:16]), unsafe)
        return jnp.maximum(bad, jnp.max(flag))

    bad = lax.fori_loop(0, H // UNROLL, fast_body, jnp.float32(0.0))

    @pl.when(bad > 0.0)
    def _():
        def norm_tile(row0):
            rows = pl.ds(pl.multiple_of(row0, 128), 128)
            return _normalize(x_ref[rows, :].astype(f32), -1).astype(bf16)

        def k_body(t, carry):
            k = jnp.dot(norm_tile(t * 128), wkv_ref[:, 0:D], preferred_element_type=f32)
            k = (k * bal_ref[0:1, :]).astype(bf16)
            for g in range(G):
                kb_ref[g, pl.ds(pl.multiple_of(t * 128, 128), 128), :] = k[:, g * 128:(g + 1) * 128]
            return carry

        lax.fori_loop(0, NS, k_body, 0)

        def q_body(t, carry):
            qt = lax.dot_general(wt_ref[D:2 * D, :], norm_tile(step * TQ + t * 128), NT,
                                 preferred_element_type=f32)
            qb_ref[:, pl.ds(pl.multiple_of(t * 128, 128), 128)] = qt
            return carry

        lax.fori_loop(0, TQ // 128, q_body, 0)

        def safe_body(h, carry):
            g = h // 8
            mine = lax.broadcasted_iota(i32, (128, TQ), 0) // DH == h % 8
            qm = jnp.where(mine, qb_ref[pl.ds(pl.multiple_of(g * 128, 128), 128), :], 0.0).astype(bf16)

            def keys(c):
                return pl.ds(pl.multiple_of(c * 256, 256), 256)

            def scores(c):
                s = jnp.dot(kb_ref[g, keys(c), :], qm, preferred_element_type=f32)
                return s * (DH ** -0.5 * LOG2E)

            def max_body(c, m):
                return jnp.maximum(m, jnp.max(scores(c), axis=0, keepdims=True))

            m = lax.fori_loop(0, S // 256, max_body, jnp.full((1, TQ), -jnp.inf, f32))

            def acc_body(c, la):
                p = jnp.exp2(scores(c) - m)
                o = jnp.dot(vt_ref[hrows(h), keys(c)], p.astype(bf16), preferred_element_type=f32)
                return la[0] + jnp.sum(p, axis=0, keepdims=True), la[1] + o

            l, acc = lax.fori_loop(0, S // 256, acc_body,
                                   (jnp.zeros((1, TQ), f32), jnp.zeros((DH, TQ), f32)))
            of_ref[hrows(h), :] = (acc * (1.0 / l)).astype(bf16)
            return carry

        lax.fori_loop(0, H, safe_body, 0)
        for it in range(2):
            ap_ref[it] = jnp.dot(wot_ref[2 * it], of_ref[256 * it:256 * it + 128, :],
                                 preferred_element_type=f32)
            ot_ref[128 * it:128 * (it + 1), :] = of_ref[256 * it + 128:256 * (it + 1), :]

    @pl.when(step == 0)
    def _():
        for cp in ffn_copies:
            cp.wait()

    NJ = TQ // TT
    wdt = wd_ref[...].T
    wodd = jnp.concatenate([wot_ref[1], wot_ref[3]], axis=1)
    ht, hnt, acts = [], [], []

    def trows(j):
        return pl.ds(pl.multiple_of(step * TQ + j * TT, TT), TT)

    for j in range(NJ):
        cs = slice(j * TT, (j + 1) * TT)
        attn = jnp.dot(wodd, ot_ref[:, cs], preferred_element_type=f32)
        attn = attn + (ap_ref[0, :, cs] + ap_ref[1, :, cs])
        ht.append(x_ref[trows(j), :].T.astype(f32) + attn)
        hnt.append(_normalize(ht[j], 0).astype(bf16))

    def down(j):
        if j == NJ - 1:
            y = lax.dot_general(acts[j], wd_ref[...], TN, preferred_element_type=f32)
            o_ref[trows(j), :] = (ht[j].T + y).astype(o_ref.dtype)
        else:
            y = jnp.dot(wdt, acts[j], preferred_element_type=f32)
            o_ref[trows(j), :] = (ht[j] + y).astype(o_ref.dtype).T
        pltpu.make_async_copy(o_ref.at[trows(j), :], o_hbm.at[trows(j), :], sem.at[3]).start()

    for j in range(NJ):
        gate = jnp.dot(wg_ref[...], hnt[j], preferred_element_type=f32)
        up = jnp.dot(wu_ref[...], hnt[j], preferred_element_type=f32)
        acts.append((jax.nn.gelu(gate, approximate=True) * up).astype(bf16))
        if j > 0:
            down(j - 1)
    down(NJ - 1)

    @pl.when(step == pl.num_programs(0) - 1)
    def _():
        pltpu.make_async_copy(o_ref, o_hbm, sem.at[3]).wait()


@jax.jit
def pallas_sequential_preLN__softmax_full_mha__geglu_ffn__prompt_kernel(
    A_x: jax.Array,
    A_wqkv: jax.Array,
    A_wo: jax.Array,
    B_x: jax.Array,
    B_w_gate: jax.Array,
    B_w_up: jax.Array,
    B_w_down: jax.Array,
):
    del B_x
    B, S, D = A_x.shape
    F = B_w_gate.shape[1]
    assert B == 1 and D == H * DH == 512 and S == 4 * TB and H == 2 * UNROLL

    out = pl.pallas_call(
        functools.partial(_kernel, S=S, D=D),
        grid=(S // TQ,),
        in_specs=[pl.BlockSpec(memory_space=pl.ANY)] * 6,
        out_specs=pl.BlockSpec(memory_space=pl.ANY),
        out_shape=jax.ShapeDtypeStruct((S, D), A_x.dtype),
        scratch_shapes=[
            pltpu.VMEM((S, D), bf16),
            pltpu.VMEM((D, 2 * D), bf16),
            pltpu.VMEM((D, D), bf16),
            pltpu.VMEM((D, D), bf16),
            pltpu.VMEM((F, D), bf16),
            pltpu.VMEM((F, D), bf16),
            pltpu.VMEM((F, D), bf16),
            pltpu.SemaphoreType.DMA((5,)),
            pltpu.VMEM((2 * D + H, D), bf16),
            pltpu.VMEM((D // 128, D, 128), bf16),
            pltpu.VMEM((TB, D), bf16),
            pltpu.VMEM((H, S, 128), i8),
            pltpu.VMEM((H, 128, S), i8),
            pltpu.VMEM((D, S), bf16),
            pltpu.VMEM((H, S), f32),
            pltpu.VMEM((H, S), f32),
            pltpu.VMEM((S // TB, H, 128), f32),
            pltpu.VMEM((2, D), f32),
            pltpu.VMEM((D // 2, TQ), bf16),
            pltpu.VMEM((2, D, TQ), f32),
            pltpu.VMEM((D, TQ), bf16),
            pltpu.VMEM((D // 128, S, 128), bf16),
            pltpu.VMEM((D, TQ), f32),
            pltpu.VMEM((8, TQ), f32),
            pltpu.VMEM((S, D), A_x.dtype),
        ],
        compiler_params=pltpu.CompilerParams(
            dimension_semantics=("arbitrary",),
            vmem_limit_bytes=100 * 1024 * 1024,
        ),
    )(A_x.reshape(S, D), A_wqkv, A_wo, B_w_gate.T, B_w_up.T, B_w_down)
    return out.reshape(B, S, D)
```
